```python
import jax
import jax.numpy as jnp

def _softmax(x, axis=-1):
    return jax.nn.softmax(x, axis=axis)
def _gelu(x):
    return jax.nn.gelu(x, approximate=True)
def _silu(x):
    return jax.nn.silu(x)
def _sigmoid(x):
    return jax.nn.sigmoid(x)
def _layernorm(x, axis=-1, eps=1e-5):
    m = jnp.mean(x, axis=axis, keepdims=True)
    v = jnp.var(x, axis=axis, keepdims=True)
    return (x - m) / jnp.sqrt(v + eps)
def _scatter_add(tgt, idx, src, axis=0):
    return tgt.at[idx].add(src)
def _segment_sum(src, seg, n):
    return jax.ops.segment_sum(src, seg, n)
class _Rng:
    def __init__(self, key):
        self._k = key
    def _next(self):
        self._k, sub = jax.random.split(self._k)
        return sub
    def normal(self, shape):
        return jax.random.normal(self._next(), shape, dtype=jnp.bfloat16)
    def randint(self, lo, hi, shape):
        return jax.random.randint(self._next(), shape, lo, hi, dtype=jnp.int32)
    def uniform(self, shape, lo=0.0, hi=1.0):
        return jax.random.uniform(self._next(), shape, jnp.bfloat16, lo, hi)
    def permutation(self, n):
        return jax.random.permutation(self._next(), n)


kernel_name = 'gated_mix__sliding_block_cached__mixer_s_mlp__decode'

def setup_inputs():
    _rng = _Rng(jax.random.key(int.from_bytes(__import__("os").urandom(4), "little")))
    _w = (lambda a: (lambda t: t.astype(jnp.bfloat16) if jnp.issubdtype(t.dtype, jnp.floating) else t)(jnp.asarray(a)))
    def _A_setup():
        B, Sq, D = 1, 1, 576
        Hq, Hkv, Sk, Dh = 32, 16, 65536, 128
        assert Hq % Hkv == 0, (Hq, Hkv)
        return {
            "x": _w((lambda *s: _rng.normal(s) * 0.05)(B, Sq, D)),
            "k_cache": _w((lambda *s: _rng.normal(s) * 0.05)(B, Hkv, Sk, Dh)),
            "v_cache": _w((lambda *s: _rng.normal(s) * 0.05)(B, Hkv, Sk, Dh)),
            "wq": _w((lambda *s: _rng.normal(s) * 0.05)(D, Hq * Dh) * (D ** -0.5)),
            "wo": _w((lambda *s: _rng.normal(s) * 0.05)(Hq * Dh, D) * ((Hq * Dh) ** -0.5)),
        }
    _A_in = _A_setup()

    def _B_setup():
        B, S, D, F = 1, 1, 576, 4608
        return {
            "x":  _w((lambda *s: _rng.normal(s) * 0.05)(B, S, D)),
            "w1": _w((lambda *s: _rng.normal(s) * 0.05)(D, D) * (D ** -0.5)),
            "w2": _w((lambda *s: _rng.normal(s) * 0.05)(D, D) * (D ** -0.5)),
            "w3": _w((lambda *s: _rng.normal(s) * 0.05)(D, F) * (D ** -0.5)),
            "w4": _w((lambda *s: _rng.normal(s) * 0.05)(F, D) * (F ** -0.5)),
        }
    _B_in = _B_setup()

    return {
        "A_x": _A_in["x"],
        "A_k_cache": _A_in["k_cache"],
        "A_v_cache": _A_in["v_cache"],
        "A_wq": _A_in["wq"],
        "A_wo": _A_in["wo"],
        "B_x": _B_in["x"],
        "B_w1": _B_in["w1"],
        "B_w2": _B_in["w2"],
        "B_w3": _B_in["w3"],
        "B_w4": _B_in["w4"],
        "gate_w": _w((lambda *s: _rng.normal(s) * 0.05)(576)),
    }

def reference(A_x, A_k_cache, A_v_cache, A_wq, A_wo, B_x, B_w1, B_w2, B_w3, B_w4, gate_w):
    def _A_ref(x, k_cache, v_cache, wq, wo):
        B, Sq, D = x.shape
        Hq, Dh = 32, 128
        Hkv, Sk = k_cache.shape[1], k_cache.shape[2]
        W = min(4096, max(256, Sk // 4))
        rep = Hq // Hkv
        q = (lambda x, *d: x.transpose(*d))((x @ wq).reshape(B, Sq, Hq, Dh), 0, 2, 1, 3)
        k = jnp.repeat(k_cache[:, :, Sk - W:, :], rep, axis=1)
        v = jnp.repeat(v_cache[:, :, Sk - W:, :], rep, axis=1)
        scores = jnp.einsum("bhqd,bhkd->bhqk", q, k) * (Dh ** -0.5)
        p = _softmax(scores, axis=-1)
        o = jnp.einsum("bhqk,bhkd->bhqd", p, v)
        return (lambda x, *d: x.transpose(*d))(o, 0, 2, 1, 3).reshape(B, Sq, Hq * Dh) @ wo

    def _B_ref(x, w1, w2, w3, w4):
        B, S, D = x.shape
        h = _gelu(_layernorm(x, axis=-1) @ w1)
        c = D // 4
        g0 = jnp.pad(h[:, :, 0*c:1*c], ((0, 0), (1, 0), (0, 0)))[:, :S, :]
        g1 = jnp.pad(h[:, :, 1*c:2*c], ((0, 0), (0, 1), (0, 0)))[:, 1:, :]
        g2 = jnp.pad(h[:, :, 2*c:3*c], ((0, 0), (2, 0), (0, 0)))[:, :S, :]
        g3 = jnp.pad(h[:, :, 3*c:   ], ((0, 0), (0, 2), (0, 0)))[:, 2:, :]
        hs = jnp.concatenate([g0, g1, g2, g3], axis=-1) @ w2
        x1 = x + hs
        h2 = _gelu(_layernorm(x1, axis=-1) @ w3) @ w4
        return x1 + h2

    x = A_x
    g = _sigmoid((x * gate_w).sum(-1, keepdims=True))
    a = _A_ref(x, A_k_cache, A_v_cache, A_wq, A_wo)
    b = _B_ref(x, B_w1, B_w2, B_w3, B_w4)
    return g * a + (1 - g) * b
```

```python
import jax
import jax.numpy as jnp
import numpy as np
from jax import lax
from jax.experimental import pallas as pl
from jax.experimental.pallas import tpu as pltpu

D, HQ, HKV, DH, F = 576, 32, 16, 128, 4608
BF16, F32 = jnp.bfloat16, jnp.float32
NT = (((1,), (1,)), ((), ()))

HEADS_PER_GROUP, HEADS_ON_Q0, KV_ROWS = 8, 2, 64
BANDS, BANDS_ON_Q0 = 9, 3
BAND_ROWS = D // BANDS
W4_COLS = (1152, 1152, 1152, 640, 384, 128)
N_GROUPS = HKV // HEADS_PER_GROUP
N_SEMS = 4 + 2 * N_GROUPS + len(W4_COLS)


def _gelu(x):
    c = np.float32(np.sqrt(2.0 / np.pi))
    return x * (0.5 * (1.0 + jnp.tanh(c * (x + 0.044715 * (x * x * x)))))


def _compute(x_hbm, gw_hbm, k_hbm, v_hbm, wq_hbm, wo_hbm, w3_hbm, w4_hbm, out_v,
             x_v, gw_v, k_v, v_v, wq_v, wo_v, w3_v, w4_v, q_v, p_v, l_v, o_v, h_v, sem):
    win = k_v.shape[1]
    start = k_hbm.shape[2] - win
    s_x, s_wq, s_w3, s_wo = (sem.at[i] for i in range(4))
    s_k = [sem.at[4 + g] for g in range(N_GROUPS)]
    s_v = [sem.at[4 + N_GROUPS + g] for g in range(N_GROUPS)]
    s_w4 = [sem.at[4 + 2 * N_GROUPS + i] for i in range(len(W4_COLS))]

    def fetch_weight(src, dst, s, col0, width, blocks):
        tile_rows = BAND_ROWS // 8

        def step(t, carry):
            rows = pl.ds(pl.multiple_of((t % tile_rows) * 8, 8), 8)
            cols = pl.ds(pl.multiple_of(col0 + (t // tile_rows) * width, 128), width)
            for queue, (lo, hi) in enumerate(((0, BANDS_ON_Q0), (BANDS_ON_Q0, BANDS))):
                idx = (pl.ds(lo, hi - lo), rows, cols)
                pltpu.make_async_copy(src.at[idx], dst.at[idx], s).start(priority=queue)
            return carry

        lax.fori_loop(0, tile_rows * blocks, step, 0)

    def fetch_cache(src, dst, s, group):
        def step(t, carry):
            row = pl.multiple_of(t * KV_ROWS, KV_ROWS)
            for queue, (lo, hi) in enumerate(((0, HEADS_ON_Q0), (HEADS_ON_Q0, HEADS_PER_GROUP))):
                heads = pl.ds(group * HEADS_PER_GROUP + lo, hi - lo)
                pltpu.make_async_copy(src.at[0, heads, pl.ds(start + row, KV_ROWS)],
                                      dst.at[heads, pl.ds(row, KV_ROWS)], s).start(priority=queue)
            return carry

        lax.fori_loop(0, win // KV_ROWS, step, 0)

    def wait(buf, s):
        pltpu.make_async_copy(buf, buf, s).wait()

    def weight(ref, cols):
        return jnp.concatenate([ref[b, :, cols] for b in range(BANDS)], axis=0)

    def group_of(ref, group):
        return ref.at[pl.ds(group * HEADS_PER_GROUP, HEADS_PER_GROUP)]

    small = [pltpu.make_async_copy(src, dst, s_x)
             for src, dst in ((x_hbm, x_v), (gw_hbm, gw_v))]
    for copy in small:
        copy.start()
    fetch_weight(wq_hbm, wq_v, s_wq, 0, 1024, HQ * DH // 1024)
    fetch_weight(w3_hbm, w3_v, s_w3, 0, 1152, F // 1152)
    fetch_cache(k_hbm, k_v, s_k[0], 0)
    for copy in small:
        copy.wait()
    wait(wq_v, s_wq)
    wait(w3_v, s_w3)

    x = x_v[0].astype(F32)
    gate = jax.nn.sigmoid(jnp.sum(x * gw_v[...].astype(F32).reshape(1, D), axis=-1, keepdims=True))
    centered = x - jnp.mean(x, axis=-1, keepdims=True)
    normed = centered / jnp.sqrt(jnp.mean(centered * centered, axis=-1, keepdims=True) + 1e-5)
    x8 = jnp.broadcast_to(x, (8, D)).astype(BF16)
    normed8 = jnp.broadcast_to(normed, (8, D)).astype(BF16)

    even = (lax.broadcasted_iota(jnp.int32, (8, DH), 0) & 1) == 0

    def q_proj(i, carry):
        cols = pl.ds(pl.multiple_of(i * 512, 512), 512)
        q = jnp.dot(x8, weight(wq_v, cols), preferred_element_type=F32)
        q_v[2 * i] = jnp.where(even, q[:, 0:128], q[:, 128:256])
        q_v[2 * i + 1] = jnp.where(even, q[:, 256:384], q[:, 384:512])
        return carry

    def mlp_up(i, carry):
        cols = pl.ds(pl.multiple_of(i * 512, 512), 512)
        h_v[:, cols] = _gelu(jnp.dot(normed8, weight(w3_v, cols), preferred_element_type=F32))
        return carry

    def scores(h, carry):
        s = lax.dot_general(q_v[h].astype(BF16), k_v[h], NT, preferred_element_type=F32) * (DH ** -0.5)
        p = jnp.exp(s - jnp.max(s, axis=-1, keepdims=True))
        l_v[h] = jnp.broadcast_to(jnp.sum(p, axis=-1, keepdims=True), (8, DH))
        p_v[h] = p
        return carry

    def values(h, carry):
        o_v[h] = jnp.dot(p_v[h].astype(BF16), v_v[h], preferred_element_type=F32) / l_v[h]
        return carry

    def o_proj(i, acc):
        o0, o1 = o_v[2 * i], o_v[2 * i + 1]
        lhs = jnp.concatenate([jnp.where(even, o0, 0.0), jnp.where(even, 0.0, o0),
                               jnp.where(even, o1, 0.0), jnp.where(even, 0.0, o1)], axis=-1).astype(BF16)
        cols = pl.ds(pl.multiple_of(i * 512, 512), 512)
        return acc + lax.dot_general(lhs, weight(wo_v, cols), NT, preferred_element_type=F32)

    lax.fori_loop(0, HQ * DH // 512, q_proj, 0)
    lax.fori_loop(0, F // 512, mlp_up, 0)

    for g in range(N_GROUPS):
        first, last = g * HEADS_PER_GROUP, (g + 1) * HEADS_PER_GROUP
        fetch_cache(v_hbm, v_v, s_v[g], g)
        wait(group_of(k_v, g), s_k[g])
        lax.fori_loop(first, last, scores, 0)
        if g + 1 < N_GROUPS:
            fetch_cache(k_hbm, k_v, s_k[g + 1], g + 1)
        else:
            fetch_weight(wo_hbm, wo_v, s_wo, 0, 1024, HQ * DH // 1024)
            col = 0
            for i, width in enumerate(W4_COLS):
                fetch_weight(w4_hbm, w4_v, s_w4[i], col, width, 1)
                col += width
        wait(group_of(v_v, g), s_v[g])
        lax.fori_loop(first, last, values, 0)

    wait(wo_v, s_wo)
    attn = lax.fori_loop(0, HQ * DH // 512, o_proj, jnp.zeros((8, D), F32))
    base = gate * (attn[0:1] + attn[1:2]) + (1.0 - gate) * x

    col, mlp = 0, None
    for i, width in enumerate(W4_COLS):
        cols = pl.ds(col, width)
        wait(w4_v.at[:, :, cols], s_w4[i])
        part = lax.dot_general(h_v[:, cols].astype(BF16), weight(w4_v, cols), NT, preferred_element_type=F32)
        mlp = part if mlp is None else mlp + part
        col += width
    out_v[0] = (base + (1.0 - gate) * mlp[0:1]).astype(out_v.dtype)


def _kernel(*refs):
    *inputs_and_scratch, out_v, out_sem = refs
    inputs, out_hbm, scratch = inputs_and_scratch[:8], inputs_and_scratch[8], inputs_and_scratch[9:]
    write_out = pltpu.make_async_copy(out_v, out_hbm, out_sem)

    def scoped(sem):
        _compute(*inputs, out_v, *scratch, sem)
        write_out.start()

    pl.run_scoped(scoped, pltpu.SemaphoreType.DMA((N_SEMS,)))
    write_out.wait()


@jax.jit
def pallas_gated_mix__sliding_block_cached__mixer_s_mlp__decode_kernel(
    A_x: jax.Array,
    A_k_cache: jax.Array,
    A_v_cache: jax.Array,
    A_wq: jax.Array,
    A_wo: jax.Array,
    B_x: jax.Array,
    B_w1: jax.Array,
    B_w2: jax.Array,
    B_w3: jax.Array,
    B_w4: jax.Array,
    gate_w: jax.Array,
):
    del B_x, B_w1, B_w2
    win = min(4096, max(256, A_k_cache.shape[2] // 4))
    hbm = pl.BlockSpec(memory_space=pl.ANY)

    def banded(w):
        return w.reshape(BANDS, BAND_ROWS, w.shape[-1])

    return pl.pallas_call(
        _kernel,
        out_shape=jax.ShapeDtypeStruct((1, 1, D), A_x.dtype),
        in_specs=[hbm] * 8,
        out_specs=hbm,
        scratch_shapes=[
            pltpu.VMEM((1, 1, D), BF16),
            pltpu.VMEM((D,), BF16),
            pltpu.VMEM((HKV, win, DH), BF16),
            pltpu.VMEM((HKV, win, DH), BF16),
            pltpu.VMEM((BANDS, BAND_ROWS, HQ * DH), BF16),
            pltpu.VMEM((BANDS, BAND_ROWS, HQ * DH), BF16),
            pltpu.VMEM((BANDS, BAND_ROWS, F), BF16),
            pltpu.VMEM((BANDS, BAND_ROWS, F), BF16),
            pltpu.VMEM((HKV, 8, DH), F32),
            pltpu.VMEM((HKV, 8, win), F32),
            pltpu.VMEM((HKV, 8, DH), F32),
            pltpu.VMEM((HKV, 8, DH), F32),
            pltpu.VMEM((8, F), F32),
            pltpu.VMEM((1, 1, D), A_x.dtype),
            pltpu.SemaphoreType.DMA(()),
        ],
        compiler_params=pltpu.CompilerParams(vmem_limit_bytes=100 * 1024 * 1024),
    )(A_x, gate_w, A_k_cache, A_v_cache,
      banded(A_wq), banded(A_wo.T), banded(B_w3), banded(B_w4.T))
```

```python
import jax
import jax.numpy as jnp
import numpy as np
from jax import lax
from jax.experimental import pallas as pl
from jax.experimental.pallas import tpu as pltpu

D, HQ, HKV, DH, F = 576, 32, 16, 128, 4608
BF16, F32 = jnp.bfloat16, jnp.float32
NT = (((1,), (1,)), ((), ()))

RING = 8
BANDS, BAND_ROWS = 9, 64
GROUP, CACHE_ROWS = 8, 64
KEYS = 512
W4_COLS = 1152
W4_LAST = ((1024, 1024), (768, 768), (1024,))
O_STEP = 4
RAMP_SPINS = 9


def _gelu(x):
    c = np.float32(np.sqrt(2.0 / np.pi))
    return x * (0.5 * (1.0 + jnp.tanh(c * (x + 0.044715 * (x * x * x)))))


def _divmod(j, n):
    if isinstance(j, int):
        return divmod(j, n)
    if n & (n - 1) == 0:
        return j >> (n.bit_length() - 1), j & (n - 1)
    scale = -(-1024 // n)
    assert all((t * scale) >> 10 == t // n for t in range(128))
    q = (j * scale) >> 10
    return q, j - q * n


def _ds(start, size, align):
    return pl.ds(start if isinstance(start, int) else pl.multiple_of(start, align), size)


def _split(src, dst, bands, first, rows, cols):
    parts = [(queue, src.at[idx], dst.at[idx]) for queue, idx in enumerate(
        ((pl.ds(0, first), rows, cols), (pl.ds(first, bands - first), rows, cols)))]
    return parts, dst.at[pl.ds(0, bands), rows, cols]


def _weight_phase(src, dst, width):
    blocks = src.shape[-1] // width

    def period(j):
        row, col = _divmod(j, blocks)
        return _split(src, dst, BANDS, 2, _ds(row * 8, 8, 8), _ds(col * width, width, 128))

    return blocks * BAND_ROWS // 8, period


def _cache_phase(src, dst, group):
    win = dst.shape[1]
    start = src.shape[2] - win

    def period(j):
        row = j * CACHE_ROWS
        rows = _ds(row, CACHE_ROWS, CACHE_ROWS)
        parts = [(queue,
                  src.at[0, pl.ds(group * GROUP + lo, hi - lo), _ds(start + row, CACHE_ROWS, CACHE_ROWS)],
                  dst.at[pl.ds(lo, hi - lo), rows])
                 for queue, (lo, hi) in enumerate(((0, 2), (2, GROUP)))]
        return parts, dst.at[:, rows]

    return win // CACHE_ROWS, period


def _w4_main_phase(src, dst):
    blocks = F // W4_COLS

    def period(j):
        t, half = _divmod(j, 2)
        row, col = _divmod(t, blocks)
        return _split(src, dst, BANDS - 1, 2, _ds((row * 2 + half) * 8, 8, 8), _ds(col * W4_COLS, W4_COLS, 128))

    return blocks * BAND_ROWS // 8, period


def _w4_last_phase(src, dst):
    widths = [w for block in W4_LAST for w in block]
    starts = np.cumsum([0] + widths).tolist()

    def period(j):
        cols = pl.ds(starts[j], widths[j])
        spans = ((1, 0, BAND_ROWS),) if j >= len(widths) - 3 else ((0, 0, 16), (1, 16, BAND_ROWS))
        parts = [(queue, src.at[BANDS - 1, pl.ds(lo, hi - lo), cols], dst.at[BANDS - 1, pl.ds(lo, hi - lo), cols])
                 for queue, lo, hi in spans]
        return parts, dst.at[BANDS - 1, :, cols]

    return len(widths), period


def _compute(x_hbm, gw_hbm, k_hbm, v_hbm, wq_hbm, wo_hbm, w3_hbm, w4_hbm, out_v,
             x_v, gw_v, k0_v, k1_v, v0_v, v1_v, wq_v, wo_v, w3_v, w4_v,
             q_v, s_v, m_v, l_v, o_v, h_v, mlp_v, spin_s, sems):
    key_blocks = k0_v.shape[1] // KEYS
    phases = [
        _weight_phase(w3_hbm, w3_v, 768),
        _weight_phase(wq_hbm, wq_v, 1024),
        _cache_phase(k_hbm, k0_v, 0),
        _cache_phase(v_hbm, v0_v, 0),
        _cache_phase(k_hbm, k1_v, 1),
        _cache_phase(v_hbm, v1_v, 1),
        _weight_phase(wo_hbm, wo_v, 1024),
        _w4_main_phase(w4_hbm, w4_v),
        _w4_last_phase(w4_hbm, w4_v),
    ]
    sizes = [n for n, _ in phases]
    firsts = np.cumsum([0] + sizes).tolist()

    def slot(position):
        return sems.at[position & (RING - 1)]

    def start(phase, j, sem):
        for queue, src, dst in phases[phase][1](j)[0]:
            pltpu.make_async_copy(src, dst, sem).start(priority=queue)

    def wait(phase, j, sem):
        region = phases[phase][1](j)[1]
        pltpu.make_async_copy(region, region, sem).wait()

    def stream(phase, step=None, lo=0, hi=None, carry=0):
        hi = sizes[phase] if hi is None else hi
        cut = sizes[phase] - RING
        for a, b, ahead, shift in ((lo, min(hi, cut), phase, RING),
                                   (max(lo, cut), hi, phase + 1, RING - sizes[phase])):
            if a < b:
                def body(j, c, ahead=ahead, shift=shift):
                    sem = slot(firsts[phase] + j)
                    wait(phase, j, sem)
                    start(ahead, j + shift, sem)
                    return c if step is None else step(j, c)
                carry = lax.fori_loop(a, b, body, carry)
        return carry

    def weight(ref, rows, cols, bands=BANDS):
        return jnp.concatenate([ref[b, rows, cols] for b in range(bands)], axis=0)

    def tile(j):
        return _ds(j * 128, 128, 128)

    small = [pltpu.make_async_copy(src, dst, sems.at[RING]) for src, dst in ((x_hbm, x_v), (gw_hbm, gw_v))]
    spin_s[0] = 0

    def spin(i, c):
        spin_s[0] = spin_s[0] + i
        return c

    for j in range(RING):
        start(0, j, slot(j))
        if j == 1:
            for copy in small:
                copy.start()
        if j >= 1:
            lax.fori_loop(0, RAMP_SPINS, spin, 0)

    stream(0, hi=sizes[0] // 2)
    for copy in small:
        copy.wait()
    x = x_v[0].astype(F32)
    gate = jax.nn.sigmoid(jnp.sum(x * gw_v[...].astype(F32).reshape(1, D), axis=-1, keepdims=True))
    centered = x - jnp.mean(x, axis=-1, keepdims=True)
    normed = centered / jnp.sqrt(jnp.mean(centered * centered, axis=-1, keepdims=True) + 1e-5)
    x8 = jnp.broadcast_to(x, (8, D)).astype(BF16)
    normed8 = jnp.broadcast_to(normed, (8, D)).astype(BF16)
    mlp_v[...] = jnp.zeros(mlp_v.shape, F32)
    stream(0, lo=sizes[0] // 2)

    def up(j):
        return jnp.dot(normed8, weight(w3_v, slice(None), tile(j)), preferred_element_type=F32)

    def up_step(j, pre):
        h_v[:, tile(j)] = _gelu(pre)
        return up(jnp.minimum(j + 1, F // 128 - 1))

    def q_step(j, c):
        q_v[j] = jnp.dot(x8, weight(wq_v, slice(None), tile(j)), preferred_element_type=F32)
        return c

    spill = F // 128 - sizes[1]
    pre = stream(1, up_step, carry=up(0))
    stream(2, lambda j, c: up_step(j + sizes[1], c), hi=spill, carry=pre)
    stream(2, lambda j, c: q_step(j - spill, c), lo=spill, hi=spill + HQ)
    stream(2, lo=spill + HQ)

    sublane = lax.broadcasted_iota(jnp.int32, (8, DH), 0)
    even = (sublane & 1) == 0

    def scores_step(group, k_v):
        def step(j, c):
            head, block = _divmod(j, key_blocks)
            keys = _ds(block * KEYS, KEYS, KEYS)
            first = 2 * (group * GROUP + head)
            q = jnp.where(even, q_v[first], q_v[first + 1]).astype(BF16)
            s = lax.dot_general(q, k_v[head, keys], NT, preferred_element_type=F32) * (DH ** -0.5)
            s_v[head, :, keys] = s
            m_v[j] = jnp.maximum(jnp.maximum(s[:, 0:128], s[:, 128:256]),
                                 jnp.maximum(s[:, 256:384], s[:, 384:512]))
            return c
        return step

    def probs(j):
        head, block = _divmod(j, key_blocks)
        row_max = jnp.max(jnp.max(m_v[_ds(head * key_blocks, key_blocks, key_blocks)], axis=0),
                          axis=-1, keepdims=True)
        return jnp.exp(s_v[head, :, _ds(block * KEYS, KEYS, KEYS)] - row_max)

    def values(phase, group, v_v, per_step):
        last = GROUP * key_blocks - 1

        def step(j, c):
            ps, o, l = c
            for u, p in enumerate(ps):
                head, block = _divmod(j * per_step + u, key_blocks)
                part = jnp.dot(p.astype(BF16), v_v[head, _ds(block * KEYS, KEYS, KEYS)],
                               preferred_element_type=F32)
                mass = (p[:, 0:128] + p[:, 128:256]) + (p[:, 256:384] + p[:, 384:512])
                if u == 0:
                    o, l = jnp.where(block == 0, part, o + part), jnp.where(block == 0, mass, l + mass)
                else:
                    o, l = o + part, l + mass
            o_v[group * GROUP + head] = o
            l_v[group * GROUP + head] = l
            return tuple(probs(jnp.minimum((j + 1) * per_step + u, last)) for u in range(per_step)), o, l

        zero = jnp.zeros((8, DH), F32)
        stream(phase, step, carry=(tuple(probs(u) for u in range(per_step)), zero, zero))

    stream(3, scores_step(0, k0_v))
    values(4, 0, v0_v, 1)
    stream(5, scores_step(1, k1_v))
    values(6, 1, v1_v, 2)

    def head_out(j):
        kv_head, which = _divmod(j, 2)
        o = o_v[kv_head] / jnp.sum(l_v[kv_head], axis=-1, keepdims=True)
        return jnp.where(sublane == which, o, 0.0).astype(BF16)

    def down_main(t):
        m, block = _divmod(t, F // W4_COLS)
        cols = _ds(block * W4_COLS, W4_COLS, 128)
        w = weight(w4_v, _ds(m * 16, 16, 16), cols, BANDS - 1)
        mlp_v[m] = mlp_v[m] + lax.dot_general(h_v[:, cols].astype(BF16), w, NT, preferred_element_type=F32)

    w4_first = firsts[7]
    o_steps = HQ // O_STEP

    def project_step(t, c):
        heads, attn = c
        sems_t = [slot(w4_first + 2 * t + u) for u in range(2)]
        wait(7, 2 * t, sems_t[0])
        wait(7, 2 * t + 1, sems_t[1])
        start(7, 2 * t + RING, sems_t[0])
        down_main(t)
        start(7, 2 * t + 1 + RING, sems_t[1])
        w = weight(wo_v, slice(None), _ds(t * O_STEP * 128, O_STEP * 128, 128))
        attn = attn + lax.dot_general(jnp.concatenate(heads, axis=1), w, NT, preferred_element_type=F32)
        ahead = jnp.minimum((t + 1) * O_STEP, HQ - O_STEP)
        return tuple(head_out(ahead + u) for u in range(O_STEP)), attn

    _, attn = lax.fori_loop(
        0, o_steps, project_step, (tuple(head_out(u) for u in range(O_STEP)), jnp.zeros((8, D), F32)))
    base = gate * (attn[0:1] + attn[1:2]) + (1.0 - gate) * x

    lane = lax.broadcasted_iota(jnp.int32, (8, 128), 1)

    def mlp_tile(t):
        out = jnp.zeros((8, 128), F32)
        for band in range(2):
            for m in range(4):
                at = 64 * band + 16 * m
                moved = pltpu.roll(mlp_v[m], (at - 16 * (2 * t + band)) % 128, 1)
                out = jnp.where((lane >= at) & (lane < at + 16), moved, out)
        return out[0:1]

    main_blocks = [[(7, 2 * t), (7, 2 * t + 1)] for t in range(o_steps, sizes[7] // 2)]
    bounds = np.cumsum([0] + [len(block) for block in W4_LAST]).tolist()
    last_blocks = [[(8, j) for j in range(a, b)] for a, b in zip(bounds, bounds[1:])]
    blocks = main_blocks[:-1] + last_blocks[:1] + main_blocks[-1:] + last_blocks[1:]
    order = [period for block in blocks for period in block]
    last_starts = np.cumsum([0] + [sum(block) for block in W4_LAST]).tolist()

    position = 0
    for block in blocks:
        for period in block:
            sem = slot(w4_first + 2 * o_steps + position)
            wait(*period, sem)
            if position + RING < len(order):
                start(*order[position + RING], sem)
            position += 1
        if block[0][0] == 7:
            down_main(block[0][1] // 2)
            continue
        i = last_blocks.index(block)
        if i == 1:
            mlp = jnp.concatenate([mlp_tile(t) for t in range(4)], axis=1)
            out_v[0, :, 0:512] = (base[:, 0:512] + (1.0 - gate) * mlp).astype(out_v.dtype)
        cols = pl.ds(last_starts[i], last_starts[i + 1] - last_starts[i])
        part = lax.dot_general(h_v[:, cols].astype(BF16), w4_v[BANDS - 1, :, cols], NT, preferred_element_type=F32)
        total = mlp_v[4, :, 0:BAND_ROWS] + part
        if block is blocks[-1]:
            out_v[0, :, 512:D] = (base[:, 512:] + (1.0 - gate) * total[0:1]).astype(out_v.dtype)
        else:
            mlp_v[4, :, 0:BAND_ROWS] = total


def _kernel(*refs):
    inputs, out_hbm, scratch, (out_v, out_sem) = refs[:8], refs[8], refs[9:-2], refs[-2:]
    write_out = pltpu.make_async_copy(out_v, out_hbm, out_sem)

    def scoped(sems):
        _compute(*inputs, out_v, *scratch, sems)
        write_out.start()

    pl.run_scoped(scoped, pltpu.SemaphoreType.DMA((RING + 1,)))
    write_out.wait()


@jax.jit
def pallas_gated_mix__sliding_block_cached__mixer_s_mlp__decode_kernel(
    A_x: jax.Array,
    A_k_cache: jax.Array,
    A_v_cache: jax.Array,
    A_wq: jax.Array,
    A_wo: jax.Array,
    B_x: jax.Array,
    B_w1: jax.Array,
    B_w2: jax.Array,
    B_w3: jax.Array,
    B_w4: jax.Array,
    gate_w: jax.Array,
):
    del B_x, B_w1, B_w2
    win = min(4096, max(256, A_k_cache.shape[2] // 4))
    key_blocks = win // KEYS
    hbm = pl.BlockSpec(memory_space=pl.ANY)

    def banded(w):
        return w.reshape(BANDS, BAND_ROWS, w.shape[-1])

    return pl.pallas_call(
        _kernel,
        out_shape=jax.ShapeDtypeStruct((1, 1, D), A_x.dtype),
        in_specs=[hbm] * 8,
        out_specs=hbm,
        scratch_shapes=[
            pltpu.VMEM((1, 1, D), BF16),
            pltpu.VMEM((D,), BF16),
            pltpu.VMEM((GROUP, win, DH), BF16),
            pltpu.VMEM((GROUP, win, DH), BF16),
            pltpu.VMEM((GROUP, win, DH), BF16),
            pltpu.VMEM((GROUP, win, DH), BF16),
            pltpu.VMEM((BANDS, BAND_ROWS, HQ * DH), BF16),
            pltpu.VMEM((BANDS, BAND_ROWS, HQ * DH), BF16),
            pltpu.VMEM((BANDS, BAND_ROWS, F), BF16),
            pltpu.VMEM((BANDS, BAND_ROWS, F), BF16),
            pltpu.VMEM((HQ, 8, DH), F32),
            pltpu.VMEM((GROUP, 8, win), F32),
            pltpu.VMEM((GROUP * key_blocks, 8, DH), F32),
            pltpu.VMEM((HKV, 8, DH), F32),
            pltpu.VMEM((HKV, 8, DH), F32),
            pltpu.VMEM((8, F), F32),
            pltpu.VMEM((5, 8, 128), F32),
            pltpu.SMEM((1,), jnp.int32),
            pltpu.VMEM((1, 1, D), A_x.dtype),
            pltpu.SemaphoreType.DMA(()),
        ],
        compiler_params=pltpu.CompilerParams(vmem_limit_bytes=100 * 1024 * 1024),
    )(A_x, gate_w, A_k_cache, A_v_cache, banded(A_wq), banded(A_wo.T), banded(B_w3), banded(B_w4.T))
```

```python
import jax
import jax.numpy as jnp
import numpy as np
from jax import lax
from jax.experimental import pallas as pl
from jax.experimental.pallas import tpu as pltpu

D, HQ, HKV, DH, F = 576, 32, 16, 128, 4608
BF16, F32 = jnp.bfloat16, jnp.float32
NT = (((1,), (1,)), ((), ()))

RING = 8
BANDS, BAND_ROWS = 9, 64
GROUP, CACHE_ROWS = 8, 64
KEYS = 512
W4_COLS = 1152
W4_LAST = ((1024, 1024), (512, 1024), (1024,))
O_STEP = 4
RAMP_SPINS = 9


def _gelu(x):
    c = np.float32(np.sqrt(2.0 / np.pi))
    return x * (0.5 * (1.0 + jnp.tanh(c * (x + 0.044715 * (x * x * x)))))


def _divmod(j, n):
    if isinstance(j, int):
        return divmod(j, n)
    if n & (n - 1) == 0:
        return j >> (n.bit_length() - 1), j & (n - 1)
    scale = -(-1024 // n)
    assert all((t * scale) >> 10 == t // n for t in range(128))
    q = (j * scale) >> 10
    return q, j - q * n


def _ds(start, size, align):
    return pl.ds(start if isinstance(start, int) else pl.multiple_of(start, align), size)


def _split(src, dst, bands, first, rows, cols):
    parts = [(queue, src.at[idx], dst.at[idx]) for queue, idx in enumerate(
        ((pl.ds(0, first), rows, cols), (pl.ds(first, bands - first), rows, cols)))]
    return parts, dst.at[pl.ds(0, bands), rows, cols]


def _weight_phase(src, dst, width, first):
    blocks = src.shape[-1] // width

    def period(j):
        row, col = _divmod(j, blocks)
        return _split(src, dst, BANDS, first, _ds(row * 8, 8, 8), _ds(col * width, width, 128))

    return blocks * BAND_ROWS // 8, period


def _cache_phase(src, dst, group):
    win = dst.shape[1]
    start = src.shape[2] - win

    def period(j):
        row = j * CACHE_ROWS
        rows = _ds(row, CACHE_ROWS, CACHE_ROWS)
        parts = [(queue,
                  src.at[0, pl.ds(group * GROUP + lo, hi - lo), _ds(start + row, CACHE_ROWS, CACHE_ROWS)],
                  dst.at[pl.ds(lo, hi - lo), rows])
                 for queue, (lo, hi) in enumerate(((0, 2), (2, GROUP)))]
        return parts, dst.at[:, rows]

    return win // CACHE_ROWS, period


def _w4_main_phase(src, dst):
    blocks = F // W4_COLS

    def period(j):
        row, col = _divmod(j, blocks)
        return _split(src, dst, BANDS - 1, 1, _ds(row * 8, 8, 8), _ds(col * W4_COLS, W4_COLS, 128))

    return blocks * BAND_ROWS // 8, period


def _w4_last_phase(src, dst):
    widths = [w for block in W4_LAST for w in block]
    starts = np.cumsum([0] + widths).tolist()

    def period(j):
        cols = pl.ds(starts[j], widths[j])
        spans = ((1, 0, BAND_ROWS),) if j >= len(widths) - 3 else ((0, 0, 16), (1, 16, BAND_ROWS))
        parts = [(queue, src.at[BANDS - 1, pl.ds(lo, hi - lo), cols], dst.at[BANDS - 1, pl.ds(lo, hi - lo), cols])
                 for queue, lo, hi in spans]
        return parts, dst.at[BANDS - 1, :, cols]

    return len(widths), period


def _compute(x_hbm, gw_hbm, k_hbm, v_hbm, wq_hbm, wo_hbm, w3_hbm, w4_hbm, out_v,
             x_v, gw_v, k0_v, k1_v, v0_v, v1_v, wq_v, wo_v, w3_v, w4_v,
             q_v, s_v, m_v, l_v, o_v, h_v, mlp_v, spin_s, sems):
    key_blocks = k0_v.shape[1] // KEYS
    phases = [
        _weight_phase(w3_hbm, w3_v, 768, 2),
        _weight_phase(wq_hbm, wq_v, 1024, 2),
        _cache_phase(k_hbm, k0_v, 0),
        _cache_phase(v_hbm, v0_v, 0),
        _cache_phase(k_hbm, k1_v, 1),
        _cache_phase(v_hbm, v1_v, 1),
        _weight_phase(wo_hbm, wo_v, 1024, 2),
        _w4_main_phase(w4_hbm, w4_v),
        _w4_last_phase(w4_hbm, w4_v),
    ]
    sizes = [n for n, _ in phases]
    firsts = np.cumsum([0] + sizes).tolist()

    def slot(position):
        return sems.at[position & (RING - 1)]

    def start(phase, j, sem):
        for queue, src, dst in phases[phase][1](j)[0]:
            pltpu.make_async_copy(src, dst, sem).start(priority=queue)

    def wait(phase, j, sem):
        region = phases[phase][1](j)[1]
        pltpu.make_async_copy(region, region, sem).wait()

    def stream(phase, step=None, lo=0, hi=None, carry=0):
        hi = sizes[phase] if hi is None else hi
        cut = sizes[phase] - RING
        for a, b, ahead, shift in ((lo, min(hi, cut), phase, RING),
                                   (max(lo, cut), hi, phase + 1, RING - sizes[phase])):
            if a < b:
                def body(j, c, ahead=ahead, shift=shift):
                    sem = slot(firsts[phase] + j)
                    wait(phase, j, sem)
                    start(ahead, j + shift, sem)
                    return c if step is None else step(j, c)
                carry = lax.fori_loop(a, b, body, carry)
        return carry

    def weight(ref, rows, cols, bands=BANDS):
        return jnp.concatenate([ref[b, rows, cols] for b in range(bands)], axis=0)

    def tile(j):
        return _ds(j * 128, 128, 128)

    small = [pltpu.make_async_copy(src, dst, sems.at[RING]) for src, dst in ((x_hbm, x_v), (gw_hbm, gw_v))]
    spin_s[0] = 0

    def spin(i, c):
        spin_s[0] = spin_s[0] + i
        return c

    for j in range(RING):
        start(0, j, slot(j))
        if j == 1:
            for copy in small:
                copy.start()
        if j >= 1:
            lax.fori_loop(0, RAMP_SPINS, spin, 0)

    stream(0, hi=sizes[0] // 2)
    for copy in small:
        copy.wait()
    x = x_v[0].astype(F32)
    gate = jax.nn.sigmoid(jnp.sum(x * gw_v[...].astype(F32).reshape(1, D), axis=-1, keepdims=True))
    centered = x - jnp.mean(x, axis=-1, keepdims=True)
    normed = centered / jnp.sqrt(jnp.mean(centered * centered, axis=-1, keepdims=True) + 1e-5)
    x8 = jnp.broadcast_to(x, (8, D)).astype(BF16)
    normed8 = jnp.broadcast_to(normed, (8, D)).astype(BF16)
    mlp_v[...] = jnp.zeros(mlp_v.shape, F32)
    stream(0, lo=sizes[0] // 2)

    def up(j):
        return jnp.dot(normed8, weight(w3_v, slice(None), tile(j)), preferred_element_type=F32)

    def up_step(j, pre):
        h_v[:, tile(j)] = _gelu(pre)
        return up(jnp.minimum(j + 1, F // 128 - 1))

    def q_step(j, c):
        q_v[j] = jnp.dot(x8, weight(wq_v, slice(None), tile(j)), preferred_element_type=F32)
        return c

    spill = F // 128 - sizes[1]
    pre = stream(1, up_step, carry=up(0))
    stream(2, lambda j, c: up_step(j + sizes[1], c), hi=spill, carry=pre)
    stream(2, lambda j, c: q_step(j - spill, c), lo=spill, hi=spill + HQ)
    stream(2, lo=spill + HQ)

    sublane = lax.broadcasted_iota(jnp.int32, (8, DH), 0)
    even = (sublane & 1) == 0

    def scores_step(group, k_v):
        def step(j, c):
            head, block = _divmod(j, key_blocks)
            keys = _ds(block * KEYS, KEYS, KEYS)
            first = 2 * (group * GROUP + head)
            q = jnp.where(even, q_v[first], q_v[first + 1]).astype(BF16)
            s = lax.dot_general(q, k_v[head, keys], NT, preferred_element_type=F32) * (DH ** -0.5)
            s_v[head, :, keys] = s
            m_v[j] = jnp.maximum(jnp.maximum(s[:, 0:128], s[:, 128:256]),
                                 jnp.maximum(s[:, 256:384], s[:, 384:512]))
            return c
        return step

    def probs(j):
        head, block = _divmod(j, key_blocks)
        row_max = jnp.max(jnp.max(m_v[_ds(head * key_blocks, key_blocks, key_blocks)], axis=0),
                          axis=-1, keepdims=True)
        return jnp.exp(s_v[head, :, _ds(block * KEYS, KEYS, KEYS)] - row_max)

    def values(phase, group, v_v, per_step):
        last = GROUP * key_blocks - 1

        def step(j, c):
            ps, o, l = c
            for u, p in enumerate(ps):
                head, block = _divmod(j * per_step + u, key_blocks)
                part = jnp.dot(p.astype(BF16), v_v[head, _ds(block * KEYS, KEYS, KEYS)],
                               preferred_element_type=F32)
                mass = (p[:, 0:128] + p[:, 128:256]) + (p[:, 256:384] + p[:, 384:512])
                if u == 0:
                    o, l = jnp.where(block == 0, part, o + part), jnp.where(block == 0, mass, l + mass)
                else:
                    o, l = o + part, l + mass
            o_v[group * GROUP + head] = o
            l_v[group * GROUP + head] = l
            return tuple(probs(jnp.minimum((j + 1) * per_step + u, last)) for u in range(per_step)), o, l

        zero = jnp.zeros((8, DH), F32)
        stream(phase, step, carry=(tuple(probs(u) for u in range(per_step)), zero, zero))

    stream(3, scores_step(0, k0_v))
    values(4, 0, v0_v, 1)
    stream(5, scores_step(1, k1_v))
    values(6, 1, v1_v, 2)

    def head_out(j):
        kv_head, which = _divmod(j, 2)
        o = o_v[kv_head] / jnp.sum(l_v[kv_head], axis=-1, keepdims=True)
        return jnp.where(sublane == which, o, 0.0).astype(BF16)

    def down_main(t):
        m, block = _divmod(t, 2)
        cols = _ds(block * 2 * W4_COLS, 2 * W4_COLS, 128)
        w = weight(w4_v, _ds(m * 8, 8, 8), cols, BANDS - 1)
        mlp_v[m, :, 0:64] = mlp_v[m, :, 0:64] + lax.dot_general(
            h_v[:, cols].astype(BF16), w, NT, preferred_element_type=F32)

    w4_first = firsts[7]
    o_steps = HQ // O_STEP

    def project_step(t, c):
        heads, attn = c
        sems_t = [slot(w4_first + 2 * t + u) for u in range(2)]
        wait(7, 2 * t, sems_t[0])
        wait(7, 2 * t + 1, sems_t[1])
        start(7, 2 * t + RING, sems_t[0])
        down_main(t)
        start(7, 2 * t + 1 + RING, sems_t[1])
        w = weight(wo_v, slice(None), _ds(t * O_STEP * 128, O_STEP * 128, 128))
        attn = attn + lax.dot_general(jnp.concatenate(heads, axis=1), w, NT, preferred_element_type=F32)
        ahead = jnp.minimum((t + 1) * O_STEP, HQ - O_STEP)
        return tuple(head_out(ahead + u) for u in range(O_STEP)), attn

    _, attn = lax.fori_loop(
        0, o_steps, project_step, (tuple(head_out(u) for u in range(O_STEP)), jnp.zeros((8, D), F32)))
    base = gate * (attn[0:1] + attn[1:2]) + (1.0 - gate) * x

    lane = lax.broadcasted_iota(jnp.int32, (8, 128), 1)

    def mlp_tile(t):
        out = jnp.zeros((8, 128), F32)
        for band in range(2):
            for m in range(8):
                at = 64 * band + 8 * m
                moved = pltpu.roll(mlp_v[m], (at - 8 * (2 * t + band)) % 128, 1)
                out = jnp.where((lane >= at) & (lane < at + 8), moved, out)
        return out[0:1]

    main_blocks = [[(7, 2 * t), (7, 2 * t + 1)] for t in range(o_steps, sizes[7] // 2)]
    bounds = np.cumsum([0] + [len(block) for block in W4_LAST]).tolist()
    last_blocks = [[(8, j) for j in range(a, b)] for a, b in zip(bounds, bounds[1:])]
    blocks = main_blocks[:-1] + last_blocks[:1] + main_blocks[-1:] + last_blocks[1:]
    order = [period for block in blocks for period in block]
    last_starts = np.cumsum([0] + [sum(block) for block in W4_LAST]).tolist()

    position = 0
    for block in blocks:
        for period in block:
            sem = slot(w4_first + 2 * o_steps + position)
            wait(*period, sem)
            if position + RING < len(order):
                start(*order[position + RING], sem)
            position += 1
        if block[0][0] == 7:
            down_main(block[0][1] // 2)
            continue
        i = last_blocks.index(block)
        if i == 1:
            mlp = jnp.concatenate([mlp_tile(t) for t in range(4)], axis=1)
            out_v[0, :, 0:512] = (base[:, 0:512] + (1.0 - gate) * mlp).astype(out_v.dtype)
        cols = pl.ds(last_starts[i], last_starts[i + 1] - last_starts[i])
        part = lax.dot_general(h_v[:, cols].astype(BF16), w4_v[BANDS - 1, :, cols], NT, preferred_element_type=F32)
        total = mlp_v[8, :, 0:BAND_ROWS] + part
        if block is blocks[-1]:
            out_v[0, :, 512:D] = (base[:, 512:] + (1.0 - gate) * total[0:1]).astype(out_v.dtype)
        else:
            mlp_v[8, :, 0:BAND_ROWS] = total


def _kernel(*refs):
    pl.run_scoped(lambda sems: _compute(*refs, sems), pltpu.SemaphoreType.DMA((RING + 1,)))


@jax.jit
def pallas_gated_mix__sliding_block_cached__mixer_s_mlp__decode_kernel(
    A_x: jax.Array,
    A_k_cache: jax.Array,
    A_v_cache: jax.Array,
    A_wq: jax.Array,
    A_wo: jax.Array,
    B_x: jax.Array,
    B_w1: jax.Array,
    B_w2: jax.Array,
    B_w3: jax.Array,
    B_w4: jax.Array,
    gate_w: jax.Array,
):
    del B_x, B_w1, B_w2
    win = min(4096, max(256, A_k_cache.shape[2] // 4))
    key_blocks = win // KEYS
    hbm = pl.BlockSpec(memory_space=pl.ANY)

    def banded(w):
        return w.reshape(BANDS, BAND_ROWS, w.shape[-1])

    return pl.pallas_call(
        _kernel,
        out_shape=jax.ShapeDtypeStruct((1, 1, D), A_x.dtype),
        in_specs=[hbm] * 8,
        out_specs=pl.BlockSpec(memory_space=pltpu.VMEM),
        scratch_shapes=[
            pltpu.VMEM((1, 1, D), BF16),
            pltpu.VMEM((D,), BF16),
            pltpu.VMEM((GROUP, win, DH), BF16),
            pltpu.VMEM((GROUP, win, DH), BF16),
            pltpu.VMEM((GROUP, win, DH), BF16),
            pltpu.VMEM((GROUP, win, DH), BF16),
            pltpu.VMEM((BANDS, BAND_ROWS, HQ * DH), BF16),
            pltpu.VMEM((BANDS, BAND_ROWS, HQ * DH), BF16),
            pltpu.VMEM((BANDS, BAND_ROWS, F), BF16),
            pltpu.VMEM((BANDS, BAND_ROWS, F), BF16),
            pltpu.VMEM((HQ, 8, DH), F32),
            pltpu.VMEM((GROUP, 8, win), F32),
            pltpu.VMEM((GROUP * key_blocks, 8, DH), F32),
            pltpu.VMEM((HKV, 8, DH), F32),
            pltpu.VMEM((HKV, 8, DH), F32),
            pltpu.VMEM((8, F), F32),
            pltpu.VMEM((9, 8, 128), F32),
            pltpu.SMEM((1,), jnp.int32),
        ],
        compiler_params=pltpu.CompilerParams(vmem_limit_bytes=100 * 1024 * 1024),
    )(A_x, gate_w, A_k_cache, A_v_cache, banded(A_wq), banded(A_wo.T), banded(B_w3), banded(B_w4.T))
```

```python
import jax
import jax.numpy as jnp
import numpy as np
from jax import lax
from jax.experimental import pallas as pl
from jax.experimental.pallas import tpu as pltpu

D, HQ, HKV, DH, F = 576, 32, 16, 128, 4608
BF16, F32 = jnp.bfloat16, jnp.float32
NT = (((1,), (1,)), ((), ()))

RING = 12
BANDS, BAND_ROWS = 9, 64
GROUP, CACHE_ROWS = 8, 64
KEYS = 512
W4_COLS = 1152
W4_LAST = ((1024, 512), (1024, 1024), (1024,))
O_STEP = 4
RAMP_SPINS = 9


def _gelu(x):
    c = np.float32(np.sqrt(2.0 / np.pi))
    return x * (0.5 * (1.0 + jnp.tanh(c * (x + 0.044715 * (x * x * x)))))


def _divmod(j, n):
    if isinstance(j, int):
        return divmod(j, n)
    if n & (n - 1) == 0:
        return j >> (n.bit_length() - 1), j & (n - 1)
    scale = -(-8192 // n)
    assert all((t * scale) >> 13 == t // n for t in range(128))
    q = (j * scale) >> 13
    return q, j - q * n


def _ds(start, size, align):
    return pl.ds(start if isinstance(start, int) else pl.multiple_of(start, align), size)


def _split(src, dst, bands, first, rows, cols):
    parts = [(queue, src.at[idx], dst.at[idx]) for queue, idx in enumerate(
        ((pl.ds(0, first), rows, cols), (pl.ds(first, bands - first), rows, cols)))]
    return parts, dst.at[pl.ds(0, bands), rows, cols]


def _weight_phase(src, dst, width, first):
    blocks = src.shape[-1] // width

    def period(j):
        row, col = _divmod(j, blocks)
        return _split(src, dst, BANDS, first, _ds(row * 8, 8, 8), _ds(col * width, width, 128))

    return blocks * BAND_ROWS // 8, period


def _cache_phase(src, dst, group):
    win = dst.shape[1]
    start = src.shape[2] - win

    def period(j):
        row = j * CACHE_ROWS
        rows = _ds(row, CACHE_ROWS, CACHE_ROWS)
        parts = [(queue,
                  src.at[0, pl.ds(group * GROUP + lo, hi - lo), _ds(start + row, CACHE_ROWS, CACHE_ROWS)],
                  dst.at[pl.ds(lo, hi - lo), rows])
                 for queue, (lo, hi) in enumerate(((0, 2), (2, GROUP)))]
        return parts, dst.at[:, rows]

    return win // CACHE_ROWS, period


def _w4_main_phase(src, dst):
    blocks = F // W4_COLS

    def period(j):
        row, col = _divmod(j, blocks)
        return _split(src, dst, BANDS - 1, 1, _ds(row * 8, 8, 8), _ds(col * W4_COLS, W4_COLS, 128))

    return blocks * BAND_ROWS // 8, period


def _w4_last_phase(src, dst):
    widths = [w for block in W4_LAST for w in block]
    starts = np.cumsum([0] + widths).tolist()

    def period(j):
        idx = (BANDS - 1, slice(None), pl.ds(starts[j], widths[j]))
        return [(1, src.at[idx], dst.at[idx])], dst.at[idx]

    return len(widths), period


def _compute(x_hbm, gw_hbm, k_hbm, v_hbm, wq_hbm, wo_hbm, w3_hbm, w4_hbm, out_v,
             x_v, gw_v, k0_v, k1_v, v0_v, v1_v, wq_v, wo_v, w3_v, w4_v,
             q_v, s_v, m_v, l_v, o_v, h_v, mlp_v, spin_s, sems):
    key_blocks = k0_v.shape[1] // KEYS
    phases = [
        _weight_phase(w3_hbm, w3_v, 768, 2),
        _weight_phase(wq_hbm, wq_v, 1024, 2),
        _cache_phase(k_hbm, k0_v, 0),
        _cache_phase(v_hbm, v0_v, 0),
        _cache_phase(k_hbm, k1_v, 1),
        _cache_phase(v_hbm, v1_v, 1),
        _weight_phase(wo_hbm, wo_v, 1024, 2),
        _w4_main_phase(w4_hbm, w4_v),
        _w4_last_phase(w4_hbm, w4_v),
    ]
    sizes = [n for n, _ in phases]
    firsts = np.cumsum([0] + sizes).tolist()

    def slot(first, j):
        return sems.at[_divmod(first % RING + j, RING)[1]]

    def start(phase, j, sem):
        for queue, src, dst in phases[phase][1](j)[0]:
            pltpu.make_async_copy(src, dst, sem).start(priority=queue)

    def wait(phase, j, sem):
        region = phases[phase][1](j)[1]
        pltpu.make_async_copy(region, region, sem).wait()

    def stream(phase, step=None, lo=0, hi=None, carry=0):
        hi = sizes[phase] if hi is None else hi
        cut = sizes[phase] - RING
        for a, b, ahead, shift in ((lo, min(hi, cut), phase, RING),
                                   (max(lo, cut), hi, phase + 1, RING - sizes[phase])):
            if a < b:
                def body(j, c, ahead=ahead, shift=shift):
                    sem = slot(firsts[phase], j)
                    wait(phase, j, sem)
                    start(ahead, j + shift, sem)
                    return c if step is None else step(j, c)
                carry = lax.fori_loop(a, b, body, carry)
        return carry

    def weight(ref, rows, cols, bands=BANDS):
        return jnp.concatenate([ref[b, rows, cols] for b in range(bands)], axis=0)

    def tile(j):
        return _ds(j * 128, 128, 128)

    small = [pltpu.make_async_copy(src, dst, sems.at[RING]) for src, dst in ((x_hbm, x_v), (gw_hbm, gw_v))]
    spin_s[0] = 0

    def spin(i, c):
        spin_s[0] = spin_s[0] + i
        return c

    for j in range(RING):
        start(0, j, slot(0, j))
        if j == 1:
            for copy in small:
                copy.start()
        if j >= 1:
            lax.fori_loop(0, RAMP_SPINS, spin, 0)

    stream(0, hi=sizes[0] // 2)
    for copy in small:
        copy.wait()
    x = x_v[0].astype(F32)
    gate = jax.nn.sigmoid(jnp.sum(x * gw_v[...].astype(F32).reshape(1, D), axis=-1, keepdims=True))
    centered = x - jnp.mean(x, axis=-1, keepdims=True)
    normed = centered / jnp.sqrt(jnp.mean(centered * centered, axis=-1, keepdims=True) + 1e-5)
    x8 = jnp.broadcast_to(x, (8, D)).astype(BF16)
    normed8 = jnp.broadcast_to(normed, (8, D)).astype(BF16)
    mlp_v[...] = jnp.zeros(mlp_v.shape, F32)
    stream(0, lo=sizes[0] // 2)

    def up(j):
        return jnp.dot(normed8, weight(w3_v, slice(None), tile(j)), preferred_element_type=F32)

    def up_step(j, pre):
        h_v[:, tile(j)] = _gelu(pre)
        return up(jnp.minimum(j + 1, F // 128 - 1))

    def q_step(j, c):
        q_v[j] = jnp.dot(x8, weight(wq_v, slice(None), tile(j)), preferred_element_type=F32)
        return c

    spill = F // 128 - sizes[1]
    pre = stream(1, up_step, carry=up(0))
    stream(2, lambda j, c: up_step(j + sizes[1], c), hi=spill, carry=pre)
    stream(2, lambda j, c: q_step(j - spill, c), lo=spill, hi=spill + HQ)
    stream(2, lo=spill + HQ)

    sublane = lax.broadcasted_iota(jnp.int32, (8, DH), 0)
    even = (sublane & 1) == 0

    def scores_step(group, k_v):
        def step(j, c):
            head, block = _divmod(j, key_blocks)
            keys = _ds(block * KEYS, KEYS, KEYS)
            first = 2 * (group * GROUP + head)
            q = jnp.where(even, q_v[first], q_v[first + 1]).astype(BF16)
            s = lax.dot_general(q, k_v[head, keys], NT, preferred_element_type=F32) * (DH ** -0.5)
            s_v[head, :, keys] = s
            m_v[j] = jnp.maximum(jnp.maximum(s[:, 0:128], s[:, 128:256]),
                                 jnp.maximum(s[:, 256:384], s[:, 384:512]))
            return c
        return step

    def probs(j):
        head, block = _divmod(j, key_blocks)
        row_max = jnp.max(jnp.max(m_v[_ds(head * key_blocks, key_blocks, key_blocks)], axis=0),
                          axis=-1, keepdims=True)
        return jnp.exp(s_v[head, :, _ds(block * KEYS, KEYS, KEYS)] - row_max)

    def values(phase, group, v_v, per_step):
        last = GROUP * key_blocks - 1

        def step(j, c):
            ps, o, l = c
            for u, p in enumerate(ps):
                head, block = _divmod(j * per_step + u, key_blocks)
                part = jnp.dot(p.astype(BF16), v_v[head, _ds(block * KEYS, KEYS, KEYS)],
                               preferred_element_type=F32)
                mass = (p[:, 0:128] + p[:, 128:256]) + (p[:, 256:384] + p[:, 384:512])
                if u == 0:
                    o, l = jnp.where(block == 0, part, o + part), jnp.where(block == 0, mass, l + mass)
                else:
                    o, l = o + part, l + mass
            o_v[group * GROUP + head] = o
            l_v[group * GROUP + head] = l
            return tuple(probs(jnp.minimum((j + 1) * per_step + u, last)) for u in range(per_step)), o, l

        zero = jnp.zeros((8, DH), F32)
        stream(phase, step, carry=(tuple(probs(u) for u in range(per_step)), zero, zero))

    stream(3, scores_step(0, k0_v))
    values(4, 0, v0_v, 1)
    stream(5, scores_step(1, k1_v))
    values(6, 1, v1_v, 2)

    def head_out(j):
        kv_head, which = _divmod(j, 2)
        o = o_v[kv_head] / jnp.sum(l_v[kv_head], axis=-1, keepdims=True)
        return jnp.where(sublane == which, o, 0.0).astype(BF16)

    def down_main(t):
        m, block = _divmod(t, 2)
        cols = _ds(block * 2 * W4_COLS, 2 * W4_COLS, 128)
        w = weight(w4_v, _ds(m * 8, 8, 8), cols, BANDS - 1)
        mlp_v[m, :, 0:64] = mlp_v[m, :, 0:64] + lax.dot_general(
            h_v[:, cols].astype(BF16), w, NT, preferred_element_type=F32)

    w4_first = firsts[7]
    o_steps = HQ // O_STEP

    def project_step(t, c):
        heads, attn = c
        sems_t = [slot(w4_first, 2 * t + u) for u in range(2)]
        wait(7, 2 * t, sems_t[0])
        wait(7, 2 * t + 1, sems_t[1])
        start(7, 2 * t + RING, sems_t[0])
        down_main(t)
        start(7, 2 * t + 1 + RING, sems_t[1])
        w = weight(wo_v, slice(None), _ds(t * O_STEP * 128, O_STEP * 128, 128))
        attn = attn + lax.dot_general(jnp.concatenate(heads, axis=1), w, NT, preferred_element_type=F32)
        ahead = jnp.minimum((t + 1) * O_STEP, HQ - O_STEP)
        return tuple(head_out(ahead + u) for u in range(O_STEP)), attn

    _, attn = lax.fori_loop(
        0, o_steps, project_step, (tuple(head_out(u) for u in range(O_STEP)), jnp.zeros((8, D), F32)))
    base = gate * (attn[0:1] + attn[1:2]) + (1.0 - gate) * x

    lane = lax.broadcasted_iota(jnp.int32, (8, 128), 1)

    def mlp_tile(t):
        out = jnp.zeros((8, 128), F32)
        for band in range(2):
            for m in range(8):
                at = 64 * band + 8 * m
                moved = pltpu.roll(mlp_v[m], (at - 8 * (2 * t + band)) % 128, 1)
                out = jnp.where((lane >= at) & (lane < at + 8), moved, out)
        return out[0:1]

    main_blocks = [[(7, 2 * t), (7, 2 * t + 1)] for t in range(o_steps, sizes[7] // 2)]
    bounds = np.cumsum([0] + [len(block) for block in W4_LAST]).tolist()
    last_blocks = [[(8, j) for j in range(a, b)] for a, b in zip(bounds, bounds[1:])]
    blocks = main_blocks[:-1] + last_blocks[:1] + main_blocks[-1:] + last_blocks[1:]
    order = [period for block in blocks for period in block]
    assert order[:RING] == [(7, 2 * o_steps + u) for u in range(RING)]
    last_starts = np.cumsum([0] + [sum(block) for block in W4_LAST]).tolist()

    position = 0
    for block in blocks:
        for period in block:
            sem = slot(w4_first + 2 * o_steps, position)
            wait(*period, sem)
            if position + RING < len(order):
                start(*order[position + RING], sem)
            position += 1
        if block[0][0] == 7:
            down_main(block[0][1] // 2)
            continue
        i = last_blocks.index(block)
        if i == 1:
            mlp = jnp.concatenate([mlp_tile(t) for t in range(4)], axis=1)
            out_v[0, :, 0:512] = (base[:, 0:512] + (1.0 - gate) * mlp).astype(out_v.dtype)
        cols = pl.ds(last_starts[i], last_starts[i + 1] - last_starts[i])
        part = lax.dot_general(h_v[:, cols].astype(BF16), w4_v[BANDS - 1, :, cols], NT, preferred_element_type=F32)
        total = mlp_v[8, :, 0:BAND_ROWS] + part
        if block is blocks[-1]:
            out_v[0, :, 512:D] = (base[:, 512:] + (1.0 - gate) * total[0:1]).astype(out_v.dtype)
        else:
            mlp_v[8, :, 0:BAND_ROWS] = total


def _kernel(*refs):
    pl.run_scoped(lambda sems: _compute(*refs, sems), pltpu.SemaphoreType.DMA((RING + 1,)))


@jax.jit
def pallas_gated_mix__sliding_block_cached__mixer_s_mlp__decode_kernel(
    A_x: jax.Array,
    A_k_cache: jax.Array,
    A_v_cache: jax.Array,
    A_wq: jax.Array,
    A_wo: jax.Array,
    B_x: jax.Array,
    B_w1: jax.Array,
    B_w2: jax.Array,
    B_w3: jax.Array,
    B_w4: jax.Array,
    gate_w: jax.Array,
):
    del B_x, B_w1, B_w2
    win = min(4096, max(256, A_k_cache.shape[2] // 4))
    key_blocks = win // KEYS
    hbm = pl.BlockSpec(memory_space=pl.ANY)

    def banded(w):
        return w.reshape(BANDS, BAND_ROWS, w.shape[-1])

    return pl.pallas_call(
        _kernel,
        out_shape=jax.ShapeDtypeStruct((1, 1, D), A_x.dtype),
        in_specs=[hbm] * 8,
        out_specs=pl.BlockSpec(memory_space=pltpu.VMEM),
        scratch_shapes=[
            pltpu.VMEM((1, 1, D), BF16),
            pltpu.VMEM((D,), BF16),
            pltpu.VMEM((GROUP, win, DH), BF16),
            pltpu.VMEM((GROUP, win, DH), BF16),
            pltpu.VMEM((GROUP, win, DH), BF16),
            pltpu.VMEM((GROUP, win, DH), BF16),
            pltpu.VMEM((BANDS, BAND_ROWS, HQ * DH), BF16),
            pltpu.VMEM((BANDS, BAND_ROWS, HQ * DH), BF16),
            pltpu.VMEM((BANDS, BAND_ROWS, F), BF16),
            pltpu.VMEM((BANDS, BAND_ROWS, F), BF16),
            pltpu.VMEM((HQ, 8, DH), F32),
            pltpu.VMEM((GROUP, 8, win), F32),
            pltpu.VMEM((GROUP * key_blocks, 8, DH), F32),
            pltpu.VMEM((HKV, 8, DH), F32),
            pltpu.VMEM((HKV, 8, DH), F32),
            pltpu.VMEM((8, F), F32),
            pltpu.VMEM((9, 8, 128), F32),
            pltpu.SMEM((1,), jnp.int32),
        ],
        compiler_params=pltpu.CompilerParams(vmem_limit_bytes=100 * 1024 * 1024),
    )(A_x, gate_w, A_k_cache, A_v_cache, banded(A_wq), banded(A_wo.T), banded(B_w3), banded(B_w4.T))
```

```python
import jax
import jax.numpy as jnp
import numpy as np
from jax import lax
from jax.experimental import pallas as pl
from jax.experimental.pallas import tpu as pltpu

D, HQ, HKV, DH, F = 576, 32, 16, 128, 4608
BF16, F32 = jnp.bfloat16, jnp.float32
NT = (((1,), (1,)), ((), ()))

RING = 16
BANDS, BAND_ROWS = 9, 64
CACHE_HEADS, CACHE_ROWS = 4, 64
KEYS = 512
W4_COLS = 768
W4_LAST = ((1024, 512), (1024, 1024), (1024,))
O_STEP = 4
RAMP_SPINS = 4


def _gelu(x):
    c = np.float32(np.sqrt(2.0 / np.pi))
    return x * (0.5 * (1.0 + jnp.tanh(c * (x + 0.044715 * (x * x * x)))))


def _divmod(j, n):
    if isinstance(j, int):
        return divmod(j, n)
    if n & (n - 1) == 0:
        return j >> (n.bit_length() - 1), j & (n - 1)
    scale = -(-65536 // n)
    assert all((t * scale) >> 16 == t // n for t in range(256))
    q = (j * scale) >> 16
    return q, j - q * n


def _ds(start, size, align):
    return pl.ds(start if isinstance(start, int) else pl.multiple_of(start, align), size)


def _split(src, dst, bands, first, rows, cols):
    parts = [(queue, src.at[idx], dst.at[idx]) for queue, idx in enumerate(
        ((pl.ds(0, first), rows, cols), (pl.ds(first, bands - first), rows, cols)))]
    return parts, dst.at[pl.ds(0, bands), rows, cols]


def _weight_phase(src, dst, width, first):
    blocks = src.shape[-1] // width

    def period(j):
        row, col = _divmod(j, blocks)
        return _split(src, dst, BANDS, first, _ds(row * 8, 8, 8), _ds(col * width, width, 128))

    return blocks * BAND_ROWS // 8, period


def _cache_phase(src, dst, half):
    keys = dst.shape[1]
    start = src.shape[2] - (2 - half) * keys
    sets = HKV // CACHE_HEADS

    def period(j):
        block, head_set = _divmod(j, sets)
        row, head = block * CACHE_ROWS, head_set * CACHE_HEADS
        rows = _ds(row, CACHE_ROWS, CACHE_ROWS)
        parts = [(queue,
                  src.at[0, pl.ds(head + lo, hi - lo), _ds(start + row, CACHE_ROWS, CACHE_ROWS)],
                  dst.at[pl.ds(head + lo, hi - lo), rows])
                 for queue, (lo, hi) in enumerate(((0, 1), (1, CACHE_HEADS)))]
        return parts, dst.at[pl.ds(head, CACHE_HEADS), rows]

    return sets * keys // CACHE_ROWS, period


def _w4_main_phase(src, dst):
    blocks = F // W4_COLS

    def period(j):
        row, col = _divmod(j, blocks)
        return _split(src, dst, BANDS - 1, 1, _ds(row * 8, 8, 8), _ds(col * W4_COLS, W4_COLS, 128))

    return blocks * BAND_ROWS // 8, period


def _w4_last_phase(src, dst):
    widths = [w for block in W4_LAST for w in block]
    starts = np.cumsum([0] + widths).tolist()

    def period(j):
        idx = (BANDS - 1, slice(None), pl.ds(starts[j], widths[j]))
        return [(1, src.at[idx], dst.at[idx])], dst.at[idx]

    return len(widths), period


def _compute(x_hbm, gw_hbm, k_hbm, v_hbm, wq_hbm, wo_hbm, w3_hbm, w4_hbm, out_v,
             x_v, gw_v, k0_v, k1_v, v0_v, v1_v, wq_v, wo_v, w3_v, w4_v,
             q_v, s_v, m_v, l_v, o_v, h_v, mlp_v, spin_s, sems):
    key_blocks = k0_v.shape[1] // KEYS
    phases = [
        _weight_phase(wq_hbm, wq_v, 512, 1),
        _weight_phase(w3_hbm, w3_v, 512, 1),
        _cache_phase(k_hbm, k0_v, 0),
        _cache_phase(k_hbm, k1_v, 1),
        _cache_phase(v_hbm, v0_v, 0),
        _cache_phase(v_hbm, v1_v, 1),
        _weight_phase(wo_hbm, wo_v, 512, 1),
        _w4_main_phase(w4_hbm, w4_v),
        _w4_last_phase(w4_hbm, w4_v),
    ]
    sizes = [n for n, _ in phases]
    firsts = np.cumsum([0] + sizes).tolist()

    def slot(first, j):
        return sems.at[_divmod(first % RING + j, RING)[1]]

    def start(phase, j, sem):
        for queue, src, dst in phases[phase][1](j)[0]:
            pltpu.make_async_copy(src, dst, sem).start(priority=queue)

    def wait(phase, j, sem):
        region = phases[phase][1](j)[1]
        pltpu.make_async_copy(region, region, sem).wait()

    def stream(phase, step=None, lo=0, hi=None, carry=0, per=1):
        hi = sizes[phase] if hi is None else hi
        cut = sizes[phase] - RING
        for a, b, ahead, shift in ((lo, min(hi, cut), phase, RING),
                                   (max(lo, cut), hi, phase + 1, RING - sizes[phase])):
            if a < b:
                def body(t, c, ahead=ahead, shift=shift):
                    for u in range(per):
                        j = t * per + u
                        sem = slot(firsts[phase], j)
                        wait(phase, j, sem)
                        start(ahead, j + shift, sem)
                    return c if step is None else step(t, c)
                assert a % per == 0 and b % per == 0
                carry = lax.fori_loop(a // per, b // per, body, carry)
        return carry

    def weight(ref, rows, cols, bands=BANDS):
        return jnp.concatenate([ref[b, rows, cols] for b in range(bands)], axis=0)

    def tile(j):
        return _ds(j * 128, 128, 128)

    small = [pltpu.make_async_copy(src, dst, sems.at[RING]) for src, dst in ((x_hbm, x_v), (gw_hbm, gw_v))]
    spin_s[0] = 0

    def spin(i, c):
        spin_s[0] = spin_s[0] + i
        return c

    for j in range(RING):
        start(0, j, slot(0, j))
        if j == 1:
            for copy in small:
                copy.start()
        if j >= 1:
            lax.fori_loop(0, RAMP_SPINS, spin, 0)

    stream(0, hi=sizes[0] // 2)
    for copy in small:
        copy.wait()
    x = x_v[0].astype(F32)
    gate = jax.nn.sigmoid(jnp.sum(x * gw_v[...].astype(F32).reshape(1, D), axis=-1, keepdims=True))
    centered = x - jnp.mean(x, axis=-1, keepdims=True)
    normed = centered / jnp.sqrt(jnp.mean(centered * centered, axis=-1, keepdims=True) + 1e-5)
    x8 = jnp.broadcast_to(x, (8, D)).astype(BF16)
    normed8 = jnp.broadcast_to(normed, (8, D)).astype(BF16)
    mlp_v[...] = jnp.zeros(mlp_v.shape, F32)
    stream(0, lo=sizes[0] // 2)

    def up(j):
        return jnp.dot(normed8, weight(w3_v, slice(None), tile(j)), preferred_element_type=F32)

    def up_step(j, pre):
        h_v[:, tile(j)] = _gelu(pre)
        return up(jnp.minimum(j + 1, F // 128 - 1))

    def q_step(j, c):
        q = jnp.dot(x8, weight(wq_v, slice(None), _ds(j * 256, 256, 128)), preferred_element_type=F32)
        q_v[2 * j] = q[:, 0:128]
        q_v[2 * j + 1] = q[:, 128:256]
        return c

    stream(1)
    stream(2, q_step, hi=2 * HKV, per=2)
    stream(2, lambda t, c: up_step(t - HKV, c), lo=2 * HKV, hi=2 * (HKV + F // 128), carry=up(0), per=2)
    stream(2, lo=2 * (HKV + F // 128))

    sublane = lax.broadcasted_iota(jnp.int32, (8, DH), 0)
    even = (sublane & 1) == 0

    def scores(phase, half, k_v):
        def step(j, c):
            head, block = _divmod(j, key_blocks)
            q = jnp.where(even, q_v[2 * head], q_v[2 * head + 1]).astype(BF16)
            s = lax.dot_general(q, k_v[head, _ds(block * KEYS, KEYS, KEYS)], NT,
                                preferred_element_type=F32) * (DH ** -0.5)
            block = block + half * key_blocks
            s_v[head, :, _ds(block * KEYS, KEYS, KEYS)] = s
            m_v[head * 2 * key_blocks + block] = jnp.maximum(jnp.maximum(s[:, 0:128], s[:, 128:256]),
                                                             jnp.maximum(s[:, 256:384], s[:, 384:512]))
            return c

        stream(phase, step, per=2)

    def values(phase, half, v_v):
        def probs(j):
            head, block = _divmod(j, key_blocks)
            peaks = m_v[_ds(head * 2 * key_blocks, 2 * key_blocks, 2 * key_blocks)]
            row_max = jnp.max(jnp.max(peaks, axis=0), axis=-1, keepdims=True)
            return jnp.exp(s_v[head, :, _ds((block + half * key_blocks) * KEYS, KEYS, KEYS)] - row_max)

        def step(j, c):
            p, o, l = c
            head, block = _divmod(j, key_blocks)
            part = jnp.dot(p.astype(BF16), v_v[head, _ds(block * KEYS, KEYS, KEYS)], preferred_element_type=F32)
            mass = (p[:, 0:128] + p[:, 128:256]) + (p[:, 256:384] + p[:, 384:512])
            o, l = jnp.where(block == 0, part, o + part), jnp.where(block == 0, mass, l + mass)
            o_v[half * HKV + head] = o
            l_v[half * HKV + head] = l
            return probs(jnp.minimum(j + 1, HKV * key_blocks - 1)), o, l

        zero = jnp.zeros((8, DH), F32)
        stream(phase, step, carry=(probs(0), zero, zero), per=2)

    scores(3, 0, k0_v)
    scores(4, 1, k1_v)
    values(5, 0, v0_v)
    values(6, 1, v1_v)

    def head_out(j):
        head, which = _divmod(j, 2)
        mass = jnp.sum(l_v[head] + l_v[HKV + head], axis=-1, keepdims=True)
        return jnp.where(sublane == which, (o_v[head] + o_v[HKV + head]) / mass, 0.0).astype(BF16)

    def down_main(t, between=(lambda: None,)):
        m, block = _divmod(t, 2)
        total = mlp_v[m, :, 0:64]
        for u, action in enumerate(between):
            cols = _ds(block * (F // 2) + u * (F // 2 // len(between)), F // 2 // len(between), 128)
            w = weight(w4_v, _ds(m * 8, 8, 8), cols, BANDS - 1)
            total = total + lax.dot_general(h_v[:, cols].astype(BF16), w, NT, preferred_element_type=F32)
            action()
        mlp_v[m, :, 0:64] = total

    w4_first = firsts[7]
    o_steps = HQ // O_STEP

    def project_step(t, c):
        heads, attn = c
        sems_t = [slot(w4_first, 3 * t + u) for u in range(3)]
        for u in range(3):
            wait(7, 3 * t + u, sems_t[u])
        start(7, 3 * t + RING, sems_t[0])
        down_main(t, [lambda u=u: start(7, 3 * t + u + RING, sems_t[u]) for u in (1, 2)])
        w = weight(wo_v, slice(None), _ds(t * O_STEP * 128, O_STEP * 128, 128))
        attn = attn + lax.dot_general(jnp.concatenate(heads, axis=1), w, NT, preferred_element_type=F32)
        ahead = jnp.minimum((t + 1) * O_STEP, HQ - O_STEP)
        return tuple(head_out(ahead + u) for u in range(O_STEP)), attn

    _, attn = lax.fori_loop(
        0, o_steps, project_step, (tuple(head_out(u) for u in range(O_STEP)), jnp.zeros((8, D), F32)))
    base = gate * (attn[0:1] + attn[1:2]) + (1.0 - gate) * x

    lane = lax.broadcasted_iota(jnp.int32, (8, 128), 1)

    def mlp_tile(t):
        out = jnp.zeros((8, 128), F32)
        for band in range(2):
            for m in range(8):
                at = 64 * band + 8 * m
                moved = pltpu.roll(mlp_v[m], (at - 8 * (2 * t + band)) % 128, 1)
                out = jnp.where((lane >= at) & (lane < at + 8), moved, out)
        return out[0:1]

    main_blocks = [[(7, 3 * t + u) for u in range(3)] for t in range(o_steps, sizes[7] // 3)]
    bounds = np.cumsum([0] + [len(block) for block in W4_LAST]).tolist()
    last_blocks = [[(8, j) for j in range(a, b)] for a, b in zip(bounds, bounds[1:])]
    blocks = main_blocks[:-1] + last_blocks[:1] + main_blocks[-1:] + last_blocks[1:]
    order = [period for block in blocks for period in block]
    assert order[:RING] == [(7, 3 * o_steps + u) for u in range(RING)]
    last_starts = np.cumsum([0] + [sum(block) for block in W4_LAST]).tolist()

    position = 0
    for block in blocks:
        for period in block:
            sem = slot(w4_first + 3 * o_steps, position)
            wait(*period, sem)
            if position + RING < len(order):
                start(*order[position + RING], sem)
            position += 1
        if block[0][0] == 7:
            down_main(block[0][1] // 3)
            continue
        i = last_blocks.index(block)
        if i == 1:
            mlp = jnp.concatenate([mlp_tile(t) for t in range(4)], axis=1)
            out_v[0, :, 0:512] = (base[:, 0:512] + (1.0 - gate) * mlp).astype(out_v.dtype)
        cols = pl.ds(last_starts[i], last_starts[i + 1] - last_starts[i])
        part = lax.dot_general(h_v[:, cols].astype(BF16), w4_v[BANDS - 1, :, cols], NT, preferred_element_type=F32)
        total = mlp_v[8, :, 0:BAND_ROWS] + part
        if block is blocks[-1]:
            out_v[0, :, 512:D] = (base[:, 512:] + (1.0 - gate) * total[0:1]).astype(out_v.dtype)
        else:
            mlp_v[8, :, 0:BAND_ROWS] = total


def _kernel(*refs):
    pl.run_scoped(lambda sems: _compute(*refs, sems), pltpu.SemaphoreType.DMA((RING + 1,)))


@jax.jit
def pallas_gated_mix__sliding_block_cached__mixer_s_mlp__decode_kernel(
    A_x: jax.Array,
    A_k_cache: jax.Array,
    A_v_cache: jax.Array,
    A_wq: jax.Array,
    A_wo: jax.Array,
    B_x: jax.Array,
    B_w1: jax.Array,
    B_w2: jax.Array,
    B_w3: jax.Array,
    B_w4: jax.Array,
    gate_w: jax.Array,
):
    del B_x, B_w1, B_w2
    win = min(4096, max(256, A_k_cache.shape[2] // 4))
    key_blocks = win // KEYS
    hbm = pl.BlockSpec(memory_space=pl.ANY)

    def banded(w):
        return w.reshape(BANDS, BAND_ROWS, w.shape[-1])

    return pl.pallas_call(
        _kernel,
        out_shape=jax.ShapeDtypeStruct((1, 1, D), A_x.dtype),
        in_specs=[hbm] * 8,
        out_specs=pl.BlockSpec(memory_space=pltpu.VMEM),
        scratch_shapes=[
            pltpu.VMEM((1, 1, D), BF16),
            pltpu.VMEM((D,), BF16),
            pltpu.VMEM((HKV, win // 2, DH), BF16),
            pltpu.VMEM((HKV, win // 2, DH), BF16),
            pltpu.VMEM((HKV, win // 2, DH), BF16),
            pltpu.VMEM((HKV, win // 2, DH), BF16),
            pltpu.VMEM((BANDS, BAND_ROWS, HQ * DH), BF16),
            pltpu.VMEM((BANDS, BAND_ROWS, HQ * DH), BF16),
            pltpu.VMEM((BANDS, BAND_ROWS, F), BF16),
            pltpu.VMEM((BANDS, BAND_ROWS, F), BF16),
            pltpu.VMEM((HQ, 8, DH), F32),
            pltpu.VMEM((HKV, 8, win), F32),
            pltpu.VMEM((HKV * key_blocks, 8, DH), F32),
            pltpu.VMEM((2 * HKV, 8, DH), F32),
            pltpu.VMEM((2 * HKV, 8, DH), F32),
            pltpu.VMEM((8, F), F32),
            pltpu.VMEM((9, 8, 128), F32),
            pltpu.SMEM((1,), jnp.int32),
        ],
        compiler_params=pltpu.CompilerParams(vmem_limit_bytes=100 * 1024 * 1024),
    )(A_x, gate_w, A_k_cache, A_v_cache, banded(A_wq), banded(A_wo.T), banded(B_w3), banded(B_w4.T))
```

```python
import jax
import jax.numpy as jnp
import numpy as np
from jax import lax
from jax.experimental import pallas as pl
from jax.experimental.pallas import tpu as pltpu

D, HQ, HKV, DH, F = 576, 32, 16, 128, 4608
BF16, F32 = jnp.bfloat16, jnp.float32
NT = (((1,), (1,)), ((), ()))

RING = 16
LEAD = (12, RING)
BANDS, BAND_ROWS = 9, 64
CACHE_HEADS, CACHE_ROWS = 4, 64
KEYS = 512
W4_COLS = 768
W4_LAST = ((1024, 512), (1024, 1024), (1024,))
O_STEP = 4
RAMP_SPINS = 4


def _gelu(x):
    c = np.float32(np.sqrt(2.0 / np.pi))
    return x * (0.5 * (1.0 + jnp.tanh(c * (x + 0.044715 * (x * x * x)))))


def _divmod(j, n):
    if isinstance(j, int):
        return divmod(j, n)
    if n & (n - 1) == 0:
        return j >> (n.bit_length() - 1), j & (n - 1)
    scale = -(-65536 // n)
    assert all((t * scale) >> 16 == t // n for t in range(256))
    q = (j * scale) >> 16
    return q, j - q * n


def _ds(start, size, align):
    return pl.ds(start if isinstance(start, int) else pl.multiple_of(start, align), size)


def _split(src, dst, bands, first, rows, cols):
    parts = [(queue, src.at[idx], dst.at[idx]) for queue, idx in enumerate(
        ((pl.ds(0, first), rows, cols), (pl.ds(first, bands - first), rows, cols)))]
    return parts, dst.at[pl.ds(0, bands), rows, cols]


def _weight_phase(src, dst, width, first):
    blocks = src.shape[-1] // width

    def period(j):
        row, col = _divmod(j, blocks)
        return _split(src, dst, BANDS, first, _ds(row * 8, 8, 8), _ds(col * width, width, 128))

    return blocks * BAND_ROWS // 8, period


def _cache_phase(src, dst, half):
    keys = dst.shape[1]
    start = src.shape[2] - (2 - half) * keys
    sets = HKV // CACHE_HEADS

    def period(j):
        block, head_set = _divmod(j, sets)
        row, head = block * CACHE_ROWS, head_set * CACHE_HEADS
        rows = _ds(row, CACHE_ROWS, CACHE_ROWS)
        parts = [(queue,
                  src.at[0, pl.ds(head + lo, hi - lo), _ds(start + row, CACHE_ROWS, CACHE_ROWS)],
                  dst.at[pl.ds(head + lo, hi - lo), rows])
                 for queue, (lo, hi) in enumerate(((0, 1), (1, CACHE_HEADS)))]
        return parts, dst.at[pl.ds(head, CACHE_HEADS), rows]

    return sets * keys // CACHE_ROWS, period


def _w4_main_phase(src, dst):
    blocks = F // W4_COLS

    def period(j):
        row, col = _divmod(j, blocks)
        return _split(src, dst, BANDS - 1, 1, _ds(row * 8, 8, 8), _ds(col * W4_COLS, W4_COLS, 128))

    return blocks * BAND_ROWS // 8, period


def _w4_last_phase(src, dst):
    widths = [w for block in W4_LAST for w in block]
    starts = np.cumsum([0] + widths).tolist()

    def period(j):
        idx = (BANDS - 1, slice(None), pl.ds(starts[j], widths[j]))
        return [(1, src.at[idx], dst.at[idx])], dst.at[idx]

    return len(widths), period


def _compute(x_hbm, gw_hbm, k_hbm, v_hbm, wq_hbm, wo_hbm, w3_hbm, w4_hbm, out_v,
             x_v, gw_v, k0_v, k1_v, v0_v, v1_v, wq_v, wo_v, w3_v, w4_v,
             q_v, s_v, m_v, l_v, o_v, h_v, mlp_v, spin_s, sems):
    key_blocks = k0_v.shape[1] // KEYS
    phases = [
        _weight_phase(wq_hbm, wq_v, 512, 1),
        _weight_phase(w3_hbm, w3_v, 512, 1),
        _cache_phase(k_hbm, k0_v, 0),
        _cache_phase(k_hbm, k1_v, 1),
        _cache_phase(v_hbm, v0_v, 0),
        _cache_phase(v_hbm, v1_v, 1),
        _weight_phase(wo_hbm, wo_v, 512, 1),
        _w4_main_phase(w4_hbm, w4_v),
        _w4_last_phase(w4_hbm, w4_v),
    ]
    sizes = [n for n, _ in phases]
    firsts = np.cumsum([0] + sizes).tolist()

    def slot(first, j):
        return sems.at[_divmod(first % RING + j, RING)[1]]

    def start(queue, phase, j, first):
        for part_queue, src, dst in phases[phase][1](j)[0]:
            if part_queue == queue:
                pltpu.make_async_copy(src, dst, slot(first, j)).start(priority=queue)

    def wait(phase, j, sem):
        region = phases[phase][1](j)[1]
        pltpu.make_async_copy(region, region, sem).wait()

    def stream(phase, step=None, lo=0, hi=None, carry=0, per=1):
        n = sizes[phase]
        hi = n if hi is None else hi
        cuts = sorted({lo, hi} | {n - lead for lead in LEAD if lo < n - lead < hi})
        for a, b in zip(cuts, cuts[1:]):
            def body(t, c, a=a):
                for u in range(per):
                    j = t * per + u
                    wait(phase, j, slot(firsts[phase], j))
                    for queue, lead in enumerate(LEAD):
                        if a < n - lead:
                            start(queue, phase, j + lead, firsts[phase])
                        else:
                            start(queue, phase + 1, j + lead - n, firsts[phase + 1])
                return c if step is None else step(t, c)

            assert a % per == 0 and b % per == 0
            carry = lax.fori_loop(a // per, b // per, body, carry)
        return carry

    def weight(ref, rows, cols, bands=BANDS):
        return jnp.concatenate([ref[b, rows, cols] for b in range(bands)], axis=0)

    def tile(j):
        return _ds(j * 128, 128, 128)

    small = [pltpu.make_async_copy(src, dst, sems.at[RING]) for src, dst in ((x_hbm, x_v), (gw_hbm, gw_v))]
    spin_s[0] = 0

    def spin(i, c):
        spin_s[0] = spin_s[0] + i
        return c

    for j in range(RING):
        for queue, lead in enumerate(LEAD):
            if j < lead:
                start(queue, 0, j, 0)
        if j == 1:
            for copy in small:
                copy.start()
        if 1 <= j < LEAD[0]:
            lax.fori_loop(0, RAMP_SPINS, spin, 0)

    stream(0, hi=sizes[0] // 2)
    for copy in small:
        copy.wait()
    x = x_v[0].astype(F32)
    gate = jax.nn.sigmoid(jnp.sum(x * gw_v[...].astype(F32).reshape(1, D), axis=-1, keepdims=True))
    centered = x - jnp.mean(x, axis=-1, keepdims=True)
    normed = centered / jnp.sqrt(jnp.mean(centered * centered, axis=-1, keepdims=True) + 1e-5)
    x8 = jnp.broadcast_to(x, (8, D)).astype(BF16)
    normed8 = jnp.broadcast_to(normed, (8, D)).astype(BF16)
    mlp_v[...] = jnp.zeros(mlp_v.shape, F32)
    stream(0, lo=sizes[0] // 2)

    def up(j):
        return jnp.dot(normed8, weight(w3_v, slice(None), tile(j)), preferred_element_type=F32)

    def up_step(j, pre):
        h_v[:, tile(j)] = _gelu(pre)
        return up(jnp.minimum(j + 1, F // 128 - 1))

    def q_step(j, c):
        q = jnp.dot(x8, weight(wq_v, slice(None), _ds(j * 256, 256, 128)), preferred_element_type=F32)
        q_v[2 * j] = q[:, 0:128]
        q_v[2 * j + 1] = q[:, 128:256]
        return c

    stream(1)
    stream(2, q_step, hi=2 * HKV, per=2)
    stream(2, lambda t, c: up_step(t - HKV, c), lo=2 * HKV, hi=2 * (HKV + F // 128), carry=up(0), per=2)
    stream(2, lo=2 * (HKV + F // 128))

    sublane = lax.broadcasted_iota(jnp.int32, (8, DH), 0)
    even = (sublane & 1) == 0

    def scores(phase, half, k_v):
        def step(j, c):
            head, block = _divmod(j, key_blocks)
            q = jnp.where(even, q_v[2 * head], q_v[2 * head + 1]).astype(BF16)
            s = lax.dot_general(q, k_v[head, _ds(block * KEYS, KEYS, KEYS)], NT,
                                preferred_element_type=F32) * (DH ** -0.5)
            block = block + half * key_blocks
            s_v[head, :, _ds(block * KEYS, KEYS, KEYS)] = s
            m_v[head * 2 * key_blocks + block] = jnp.maximum(jnp.maximum(s[:, 0:128], s[:, 128:256]),
                                                             jnp.maximum(s[:, 256:384], s[:, 384:512]))
            return c

        stream(phase, step, per=2)

    def values(phase, half, v_v):
        def probs(j):
            head, block = _divmod(j, key_blocks)
            peaks = m_v[_ds(head * 2 * key_blocks, 2 * key_blocks, 2 * key_blocks)]
            row_max = jnp.max(jnp.max(peaks, axis=0), axis=-1, keepdims=True)
            return jnp.exp(s_v[head, :, _ds((block + half * key_blocks) * KEYS, KEYS, KEYS)] - row_max)

        def step(j, c):
            p, o, l = c
            head, block = _divmod(j, key_blocks)
            part = jnp.dot(p.astype(BF16), v_v[head, _ds(block * KEYS, KEYS, KEYS)], preferred_element_type=F32)
            mass = (p[:, 0:128] + p[:, 128:256]) + (p[:, 256:384] + p[:, 384:512])
            o, l = jnp.where(block == 0, part, o + part), jnp.where(block == 0, mass, l + mass)
            o_v[half * HKV + head] = o
            l_v[half * HKV + head] = l
            return probs(jnp.minimum(j + 1, HKV * key_blocks - 1)), o, l

        zero = jnp.zeros((8, DH), F32)
        stream(phase, step, carry=(probs(0), zero, zero), per=2)

    scores(3, 0, k0_v)
    scores(4, 1, k1_v)
    values(5, 0, v0_v)
    values(6, 1, v1_v)

    def head_out(j):
        head, which = _divmod(j, 2)
        mass = jnp.sum(l_v[head] + l_v[HKV + head], axis=-1, keepdims=True)
        return jnp.where(sublane == which, (o_v[head] + o_v[HKV + head]) / mass, 0.0).astype(BF16)

    def down_main(t, between=(lambda: None,)):
        m, block = _divmod(t, 2)
        total = mlp_v[m, :, 0:64]
        for u, action in enumerate(between):
            cols = _ds(block * (F // 2) + u * (F // 2 // len(between)), F // 2 // len(between), 128)
            w = weight(w4_v, _ds(m * 8, 8, 8), cols, BANDS - 1)
            total = total + lax.dot_general(h_v[:, cols].astype(BF16), w, NT, preferred_element_type=F32)
            action()
        mlp_v[m, :, 0:64] = total

    w4_first = firsts[7]
    o_steps = HQ // O_STEP

    def project_step(t, c):
        heads, attn = c
        sems_t = [slot(w4_first, 3 * t + u) for u in range(3)]
        for u in range(3):
            wait(7, 3 * t + u, sems_t[u])

        def refill(u):
            for queue, lead in enumerate(LEAD):
                start(queue, 7, 3 * t + u + lead, w4_first)

        refill(0)
        down_main(t, [lambda u=u: refill(u) for u in (1, 2)])
        w = weight(wo_v, slice(None), _ds(t * O_STEP * 128, O_STEP * 128, 128))
        attn = attn + lax.dot_general(jnp.concatenate(heads, axis=1), w, NT, preferred_element_type=F32)
        ahead = jnp.minimum((t + 1) * O_STEP, HQ - O_STEP)
        return tuple(head_out(ahead + u) for u in range(O_STEP)), attn

    _, attn = lax.fori_loop(
        0, o_steps, project_step, (tuple(head_out(u) for u in range(O_STEP)), jnp.zeros((8, D), F32)))
    base = gate * (attn[0:1] + attn[1:2]) + (1.0 - gate) * x

    lane = lax.broadcasted_iota(jnp.int32, (8, 128), 1)

    def mlp_tile(t):
        out = jnp.zeros((8, 128), F32)
        for band in range(2):
            for m in range(8):
                at = 64 * band + 8 * m
                moved = pltpu.roll(mlp_v[m], (at - 8 * (2 * t + band)) % 128, 1)
                out = jnp.where((lane >= at) & (lane < at + 8), moved, out)
        return out[0:1]

    main_blocks = [[(7, 3 * t + u) for u in range(3)] for t in range(o_steps, sizes[7] // 3)]
    bounds = np.cumsum([0] + [len(block) for block in W4_LAST]).tolist()
    last_blocks = [[(8, j) for j in range(a, b)] for a, b in zip(bounds, bounds[1:])]
    blocks = main_blocks[:-1] + last_blocks[:1] + main_blocks[-1:] + last_blocks[1:]
    order = [period for block in blocks for period in block]
    assert order[:RING] == [(7, 3 * o_steps + u) for u in range(RING)]
    last_starts = np.cumsum([0] + [sum(block) for block in W4_LAST]).tolist()

    position = 0
    for block in blocks:
        for period in block:
            sem = slot(w4_first + 3 * o_steps, position)
            wait(*period, sem)
            for queue, lead in enumerate(LEAD):
                if position + lead < len(order):
                    ahead, j = order[position + lead]
                    start(queue, ahead, j, w4_first + 3 * o_steps + position + lead - j)
            position += 1
        if block[0][0] == 7:
            down_main(block[0][1] // 3)
            continue
        i = last_blocks.index(block)
        if i == 1:
            mlp = jnp.concatenate([mlp_tile(t) for t in range(4)], axis=1)
            out_v[0, :, 0:512] = (base[:, 0:512] + (1.0 - gate) * mlp).astype(out_v.dtype)
        cols = pl.ds(last_starts[i], last_starts[i + 1] - last_starts[i])
        part = lax.dot_general(h_v[:, cols].astype(BF16), w4_v[BANDS - 1, :, cols], NT, preferred_element_type=F32)
        total = mlp_v[8, :, 0:BAND_ROWS] + part
        if block is blocks[-1]:
            out_v[0, :, 512:D] = (base[:, 512:] + (1.0 - gate) * total[0:1]).astype(out_v.dtype)
        else:
            mlp_v[8, :, 0:BAND_ROWS] = total


def _kernel(*refs):
    pl.run_scoped(lambda sems: _compute(*refs, sems), pltpu.SemaphoreType.DMA((RING + 1,)))


@jax.jit
def pallas_gated_mix__sliding_block_cached__mixer_s_mlp__decode_kernel(
    A_x: jax.Array,
    A_k_cache: jax.Array,
    A_v_cache: jax.Array,
    A_wq: jax.Array,
    A_wo: jax.Array,
    B_x: jax.Array,
    B_w1: jax.Array,
    B_w2: jax.Array,
    B_w3: jax.Array,
    B_w4: jax.Array,
    gate_w: jax.Array,
):
    del B_x, B_w1, B_w2
    win = min(4096, max(256, A_k_cache.shape[2] // 4))
    key_blocks = win // KEYS
    hbm = pl.BlockSpec(memory_space=pl.ANY)

    def banded(w):
        return w.reshape(BANDS, BAND_ROWS, w.shape[-1])

    return pl.pallas_call(
        _kernel,
        out_shape=jax.ShapeDtypeStruct((1, 1, D), A_x.dtype),
        in_specs=[hbm] * 8,
        out_specs=pl.BlockSpec(memory_space=pltpu.VMEM),
        scratch_shapes=[
            pltpu.VMEM((1, 1, D), BF16),
            pltpu.VMEM((D,), BF16),
            pltpu.VMEM((HKV, win // 2, DH), BF16),
            pltpu.VMEM((HKV, win // 2, DH), BF16),
            pltpu.VMEM((HKV, win // 2, DH), BF16),
            pltpu.VMEM((HKV, win // 2, DH), BF16),
            pltpu.VMEM((BANDS, BAND_ROWS, HQ * DH), BF16),
            pltpu.VMEM((BANDS, BAND_ROWS, HQ * DH), BF16),
            pltpu.VMEM((BANDS, BAND_ROWS, F), BF16),
            pltpu.VMEM((BANDS, BAND_ROWS, F), BF16),
            pltpu.VMEM((HQ, 8, DH), F32),
            pltpu.VMEM((HKV, 8, win), F32),
            pltpu.VMEM((HKV * key_blocks, 8, DH), F32),
            pltpu.VMEM((2 * HKV, 8, DH), F32),
            pltpu.VMEM((2 * HKV, 8, DH), F32),
            pltpu.VMEM((8, F), F32),
            pltpu.VMEM((9, 8, 128), F32),
            pltpu.SMEM((1,), jnp.int32),
        ],
        compiler_params=pltpu.CompilerParams(vmem_limit_bytes=100 * 1024 * 1024),
    )(A_x, gate_w, A_k_cache, A_v_cache, banded(A_wq), banded(A_wo.T), banded(B_w3), banded(B_w4.T))
```

```python
import jax
import jax.numpy as jnp
import numpy as np
from jax import lax
from jax.experimental import pallas as pl
from jax.experimental.pallas import tpu as pltpu

D, HQ, HKV, DH, F = 576, 32, 16, 128, 4608
BF16, F32 = jnp.bfloat16, jnp.float32
NT = (((1,), (1,)), ((), ()))

RING = 16
LEAD = (12, RING)
BANDS, BAND_ROWS = 9, 64
CACHE_HEADS, CACHE_ROWS = 4, 64
KEYS = 512
W4_COLS = 768
W4_LAST = ((1024, 512), (1024, 1024), (1024,))
O_STEP = 4
RAMP_SPINS = 4


def _gelu(x):
    c = np.float32(np.sqrt(2.0 / np.pi))
    return x * (0.5 * (1.0 + jnp.tanh(c * (x + 0.044715 * (x * x * x)))))


def _divmod(j, n):
    if isinstance(j, int):
        return divmod(j, n)
    if n & (n - 1) == 0:
        return j >> (n.bit_length() - 1), j & (n - 1)
    scale = -(-65536 // n)
    assert all((t * scale) >> 16 == t // n for t in range(256))
    q = (j * scale) >> 16
    return q, j - q * n


def _ds(start, size, align):
    return pl.ds(start if isinstance(start, int) else pl.multiple_of(start, align), size)


def _split(src, dst, bands, first, rows, cols):
    parts = [(queue, src.at[idx], dst.at[idx]) for queue, idx in enumerate(
        ((pl.ds(0, first), rows, cols), (pl.ds(first, bands - first), rows, cols)))]
    return parts, dst.at[pl.ds(0, bands), rows, cols]


def _weight_phase(src, dst, width, first):
    blocks = src.shape[-1] // width

    def period(j):
        row, col = _divmod(j, blocks)
        return _split(src, dst, BANDS, first, _ds(row * 8, 8, 8), _ds(col * width, width, 128))

    return blocks * BAND_ROWS // 8, period


def _cache_phase(src, dst, half):
    keys = dst.shape[1]
    start = src.shape[2] - (2 - half) * keys
    sets = HKV // CACHE_HEADS

    def period(j):
        block, head_set = _divmod(j, sets)
        row, head = block * CACHE_ROWS, head_set * CACHE_HEADS
        rows = _ds(row, CACHE_ROWS, CACHE_ROWS)
        parts = [(queue,
                  src.at[0, pl.ds(head + lo, hi - lo), _ds(start + row, CACHE_ROWS, CACHE_ROWS)],
                  dst.at[pl.ds(head + lo, hi - lo), rows])
                 for queue, (lo, hi) in enumerate(((0, 1), (1, CACHE_HEADS)))]
        return parts, dst.at[pl.ds(head, CACHE_HEADS), rows]

    return sets * keys // CACHE_ROWS, period


def _w4_main_phase(src, dst):
    blocks = F // W4_COLS

    def period(j):
        row, col = _divmod(j, blocks)
        return _split(src, dst, BANDS - 1, 1, _ds(row * 8, 8, 8), _ds(col * W4_COLS, W4_COLS, 128))

    return blocks * BAND_ROWS // 8, period


def _w4_last_phase(src, dst):
    widths = [w for block in W4_LAST for w in block]
    starts = np.cumsum([0] + widths).tolist()

    def period(j):
        idx = (BANDS - 1, slice(None), pl.ds(starts[j], widths[j]))
        return [(1, src.at[idx], dst.at[idx])], dst.at[idx]

    return len(widths), period


def _compute(x_hbm, gw_hbm, k_hbm, v_hbm, wq_hbm, wo_hbm, w3_hbm, w4_hbm, out_v,
             x_v, gw_v, k0_v, k1_v, v0_v, v1_v, wq_v, wo_v, w3_v, w4_v,
             q_v, s_v, m_v, l_v, o_v, h_v, mlp_v, spin_s, sems):
    key_blocks = k0_v.shape[1] // KEYS
    phases = [
        _weight_phase(wq_hbm, wq_v, 512, 1),
        _weight_phase(w3_hbm, w3_v, 512, 1),
        _cache_phase(k_hbm, k0_v, 0),
        _cache_phase(k_hbm, k1_v, 1),
        _cache_phase(v_hbm, v0_v, 0),
        _cache_phase(v_hbm, v1_v, 1),
        _weight_phase(wo_hbm, wo_v, 512, 1),
        _w4_main_phase(w4_hbm, w4_v),
        _w4_last_phase(w4_hbm, w4_v),
    ]
    sizes = [n for n, _ in phases]
    firsts = np.cumsum([0] + sizes).tolist()

    def slot(first, j):
        return sems.at[_divmod(first % RING + j, RING)[1]]

    def start(queue, phase, j, first):
        for part_queue, src, dst in phases[phase][1](j)[0]:
            if part_queue == queue:
                pltpu.make_async_copy(src, dst, slot(first, j)).start(priority=queue)

    def wait(phase, j, sem):
        region = phases[phase][1](j)[1]
        pltpu.make_async_copy(region, region, sem).wait()

    def stream(phase, step=None, lo=0, hi=None, carry=0, per=1):
        n = sizes[phase]
        hi = n if hi is None else hi
        cuts = sorted({lo, hi} | {n - lead for lead in LEAD if lo < n - lead < hi})
        for a, b in zip(cuts, cuts[1:]):
            def body(t, c, a=a):
                for u in range(per):
                    j = t * per + u
                    wait(phase, j, slot(firsts[phase], j))
                    for queue, lead in enumerate(LEAD):
                        if a < n - lead:
                            start(queue, phase, j + lead, firsts[phase])
                        else:
                            start(queue, phase + 1, j + lead - n, firsts[phase + 1])
                return c if step is None else step(t, c)

            assert a % per == 0 and b % per == 0
            carry = lax.fori_loop(a // per, b // per, body, carry)
        return carry

    def weight(ref, rows, cols, bands=BANDS):
        return jnp.concatenate([ref[b, rows, cols] for b in range(bands)], axis=0)

    def tile(j):
        return _ds(j * 128, 128, 128)

    small = [pltpu.make_async_copy(src, dst, sems.at[RING]) for src, dst in ((x_hbm, x_v), (gw_hbm, gw_v))]
    spin_s[0] = 0

    def spin(i, c):
        spin_s[0] = spin_s[0] + i
        return c

    for j in range(RING):
        for queue, lead in enumerate(LEAD):
            if j < lead:
                start(queue, 0, j, 0)
        if j == 1:
            for copy in small:
                copy.start()
        if 1 <= j < LEAD[0]:
            lax.fori_loop(0, RAMP_SPINS, spin, 0)

    stream(0, hi=sizes[0] // 2)
    for copy in small:
        copy.wait()
    x = x_v[0].astype(F32)
    gate = jax.nn.sigmoid(jnp.sum(x * gw_v[...].astype(F32).reshape(1, D), axis=-1, keepdims=True))
    centered = x - jnp.mean(x, axis=-1, keepdims=True)
    normed = centered / jnp.sqrt(jnp.mean(centered * centered, axis=-1, keepdims=True) + 1e-5)
    x8 = jnp.broadcast_to(x, (8, D)).astype(BF16)
    normed8 = jnp.broadcast_to(normed, (8, D)).astype(BF16)
    mlp_v[...] = jnp.zeros(mlp_v.shape, F32)
    stream(0, lo=sizes[0] // 2)

    def up(j):
        return jnp.dot(normed8, weight(w3_v, slice(None), tile(j)), preferred_element_type=F32)

    def up_step(j, pre):
        h_v[:, tile(j)] = _gelu(pre)
        return up(jnp.minimum(j + 1, F // 128 - 1))

    def q_step(j, c):
        q = jnp.dot(x8, weight(wq_v, slice(None), _ds(j * 256, 256, 128)), preferred_element_type=F32)
        q_v[2 * j] = q[:, 0:128]
        q_v[2 * j + 1] = q[:, 128:256]
        return c

    stream(1)
    stream(2, q_step, hi=2 * HKV, per=2)
    stream(2, lambda t, c: up_step(t - HKV, c), lo=2 * HKV, hi=2 * (HKV + F // 128), carry=up(0), per=2)
    stream(2, lo=2 * (HKV + F // 128))

    sublane = lax.broadcasted_iota(jnp.int32, (8, DH), 0)
    even = (sublane & 1) == 0

    def scores(phase, half, k_v):
        def step(j, c):
            head, block = _divmod(j, key_blocks)
            q = jnp.where(even, q_v[2 * head], q_v[2 * head + 1]).astype(BF16)
            s = lax.dot_general(q, k_v[head, _ds(block * KEYS, KEYS, KEYS)], NT,
                                preferred_element_type=F32) * (DH ** -0.5)
            block = block + half * key_blocks
            s_v[head, :, _ds(block * KEYS, KEYS, KEYS)] = s
            m_v[head * 2 * key_blocks + block] = jnp.maximum(jnp.maximum(s[:, 0:128], s[:, 128:256]),
                                                             jnp.maximum(s[:, 256:384], s[:, 384:512]))
            return c

        assert sizes[phase] == 2 * HKV * key_blocks
        stream(phase, step, per=2)

    def values(phase, half, v_v):
        total = HKV * key_blocks
        per_step = total // (sizes[phase] // 2)
        assert per_step * (sizes[phase] // 2) == total and key_blocks % per_step == 0

        def probs(j):
            head, block = _divmod(j, key_blocks)
            peaks = m_v[_ds(head * 2 * key_blocks, 2 * key_blocks, 2 * key_blocks)]
            row_max = jnp.max(jnp.max(peaks, axis=0), axis=-1, keepdims=True)
            return jnp.exp(s_v[head, :, _ds((block + half * key_blocks) * KEYS, KEYS, KEYS)] - row_max)

        def step(t, c):
            ps, o, l = c
            for u, p in enumerate(ps):
                head, block = _divmod(t * per_step + u, key_blocks)
                part = jnp.dot(p.astype(BF16), v_v[head, _ds(block * KEYS, KEYS, KEYS)],
                               preferred_element_type=F32)
                mass = (p[:, 0:128] + p[:, 128:256]) + (p[:, 256:384] + p[:, 384:512])
                if u == 0:
                    o, l = jnp.where(block == 0, part, o + part), jnp.where(block == 0, mass, l + mass)
                else:
                    o, l = o + part, l + mass
            o_v[half * HKV + head] = o
            l_v[half * HKV + head] = l
            return tuple(probs(jnp.minimum((t + 1) * per_step + u, total - 1)) for u in range(per_step)), o, l

        zero = jnp.zeros((8, DH), F32)
        stream(phase, step, carry=(tuple(probs(u) for u in range(per_step)), zero, zero), per=2)

    scores(3, 0, k0_v)
    scores(4, 1, k1_v)
    values(5, 0, v0_v)
    values(6, 1, v1_v)

    def head_out(j):
        head, which = _divmod(j, 2)
        mass = jnp.sum(l_v[head] + l_v[HKV + head], axis=-1, keepdims=True)
        return jnp.where(sublane == which, (o_v[head] + o_v[HKV + head]) / mass, 0.0).astype(BF16)

    def down_main(t, between=(lambda: None,)):
        m, block = _divmod(t, 2)
        total = mlp_v[m, :, 0:64]
        for u, action in enumerate(between):
            cols = _ds(block * (F // 2) + u * (F // 2 // len(between)), F // 2 // len(between), 128)
            w = weight(w4_v, _ds(m * 8, 8, 8), cols, BANDS - 1)
            total = total + lax.dot_general(h_v[:, cols].astype(BF16), w, NT, preferred_element_type=F32)
            action()
        mlp_v[m, :, 0:64] = total

    w4_first = firsts[7]
    o_steps = HQ // O_STEP

    def project_step(t, c):
        heads, attn = c
        sems_t = [slot(w4_first, 3 * t + u) for u in range(3)]
        for u in range(3):
            wait(7, 3 * t + u, sems_t[u])

        def refill(u):
            for queue, lead in enumerate(LEAD):
                start(queue, 7, 3 * t + u + lead, w4_first)

        refill(0)
        down_main(t, [lambda u=u: refill(u) for u in (1, 2)])
        w = weight(wo_v, slice(None), _ds(t * O_STEP * 128, O_STEP * 128, 128))
        attn = attn + lax.dot_general(jnp.concatenate(heads, axis=1), w, NT, preferred_element_type=F32)
        ahead = jnp.minimum((t + 1) * O_STEP, HQ - O_STEP)
        return tuple(head_out(ahead + u) for u in range(O_STEP)), attn

    _, attn = lax.fori_loop(
        0, o_steps, project_step, (tuple(head_out(u) for u in range(O_STEP)), jnp.zeros((8, D), F32)))
    base = gate * (attn[0:1] + attn[1:2]) + (1.0 - gate) * x

    lane = lax.broadcasted_iota(jnp.int32, (8, 128), 1)

    def mlp_tile(t):
        out = jnp.zeros((8, 128), F32)
        for band in range(2):
            for m in range(8):
                at = 64 * band + 8 * m
                moved = pltpu.roll(mlp_v[m], (at - 8 * (2 * t + band)) % 128, 1)
                out = jnp.where((lane >= at) & (lane < at + 8), moved, out)
        return out[0:1]

    main_blocks = [[(7, 3 * t + u) for u in range(3)] for t in range(o_steps, sizes[7] // 3)]
    bounds = np.cumsum([0] + [len(block) for block in W4_LAST]).tolist()
    last_blocks = [[(8, j) for j in range(a, b)] for a, b in zip(bounds, bounds[1:])]
    blocks = main_blocks[:-1] + last_blocks[:1] + main_blocks[-1:] + last_blocks[1:]
    order = [period for block in blocks for period in block]
    assert order[:RING] == [(7, 3 * o_steps + u) for u in range(RING)]
    last_starts = np.cumsum([0] + [sum(block) for block in W4_LAST]).tolist()

    position = 0
    for block in blocks:
        for period in block:
            sem = slot(w4_first + 3 * o_steps, position)
            wait(*period, sem)
            for queue, lead in enumerate(LEAD):
                if position + lead < len(order):
                    ahead, j = order[position + lead]
                    start(queue, ahead, j, w4_first + 3 * o_steps + position + lead - j)
            position += 1
        if block[0][0] == 7:
            down_main(block[0][1] // 3)
            continue
        i = last_blocks.index(block)
        if i == 1:
            mlp = jnp.concatenate([mlp_tile(t) for t in range(4)], axis=1)
            out_v[0, :, 0:512] = (base[:, 0:512] + (1.0 - gate) * mlp).astype(out_v.dtype)
        cols = pl.ds(last_starts[i], last_starts[i + 1] - last_starts[i])
        part = lax.dot_general(h_v[:, cols].astype(BF16), w4_v[BANDS - 1, :, cols], NT, preferred_element_type=F32)
        total = mlp_v[8, :, 0:BAND_ROWS] + part
        if block is blocks[-1]:
            out_v[0, :, 512:D] = (base[:, 512:] + (1.0 - gate) * total[0:1]).astype(out_v.dtype)
        else:
            mlp_v[8, :, 0:BAND_ROWS] = total


def _kernel(*refs):
    pl.run_scoped(lambda sems: _compute(*refs, sems), pltpu.SemaphoreType.DMA((RING + 1,)))


@jax.jit
def pallas_gated_mix__sliding_block_cached__mixer_s_mlp__decode_kernel(
    A_x: jax.Array,
    A_k_cache: jax.Array,
    A_v_cache: jax.Array,
    A_wq: jax.Array,
    A_wo: jax.Array,
    B_x: jax.Array,
    B_w1: jax.Array,
    B_w2: jax.Array,
    B_w3: jax.Array,
    B_w4: jax.Array,
    gate_w: jax.Array,
):
    del B_x, B_w1, B_w2
    win = min(4096, max(256, A_k_cache.shape[2] // 4))
    key_blocks = win // KEYS
    hbm = pl.BlockSpec(memory_space=pl.ANY)

    def banded(w):
        return w.reshape(BANDS, BAND_ROWS, w.shape[-1])

    return pl.pallas_call(
        _kernel,
        out_shape=jax.ShapeDtypeStruct((1, 1, D), A_x.dtype),
        in_specs=[hbm] * 8,
        out_specs=pl.BlockSpec(memory_space=pltpu.VMEM),
        scratch_shapes=[
            pltpu.VMEM((1, 1, D), BF16),
            pltpu.VMEM((D,), BF16),
            pltpu.VMEM((HKV, win // 2, DH), BF16),
            pltpu.VMEM((HKV, win // 2, DH), BF16),
            pltpu.VMEM((HKV, win // 2, DH), BF16),
            pltpu.VMEM((HKV, win // 2, DH), BF16),
            pltpu.VMEM((BANDS, BAND_ROWS, HQ * DH), BF16),
            pltpu.VMEM((BANDS, BAND_ROWS, HQ * DH), BF16),
            pltpu.VMEM((BANDS, BAND_ROWS, F), BF16),
            pltpu.VMEM((BANDS, BAND_ROWS, F), BF16),
            pltpu.VMEM((HQ, 8, DH), F32),
            pltpu.VMEM((HKV, 8, win), F32),
            pltpu.VMEM((HKV * key_blocks, 8, DH), F32),
            pltpu.VMEM((2 * HKV, 8, DH), F32),
            pltpu.VMEM((2 * HKV, 8, DH), F32),
            pltpu.VMEM((8, F), F32),
            pltpu.VMEM((9, 8, 128), F32),
            pltpu.SMEM((1,), jnp.int32),
        ],
        compiler_params=pltpu.CompilerParams(vmem_limit_bytes=100 * 1024 * 1024),
    )(A_x, gate_w, A_k_cache, A_v_cache, banded(A_wq), banded(A_wo.T), banded(B_w3), banded(B_w4.T))
```
